```python
import jax
import jax.numpy as jnp

def _softmax(x, axis=-1):
    return jax.nn.softmax(x, axis=axis)
def _gelu(x):
    return jax.nn.gelu(x, approximate=True)
def _silu(x):
    return jax.nn.silu(x)
def _sigmoid(x):
    return jax.nn.sigmoid(x)
def _layernorm(x, axis=-1, eps=1e-5):
    m = jnp.mean(x, axis=axis, keepdims=True)
    v = jnp.var(x, axis=axis, keepdims=True)
    return (x - m) / jnp.sqrt(v + eps)
def _scatter_add(tgt, idx, src, axis=0):
    return tgt.at[idx].add(src)
def _segment_sum(src, seg, n):
    return jax.ops.segment_sum(src, seg, n)
class _Rng:
    def __init__(self, key):
        self._k = key
    def _next(self):
        self._k, sub = jax.random.split(self._k)
        return sub
    def normal(self, shape):
        return jax.random.normal(self._next(), shape, dtype=jnp.bfloat16)
    def randint(self, lo, hi, shape):
        return jax.random.randint(self._next(), shape, lo, hi, dtype=jnp.int32)
    def uniform(self, shape, lo=0.0, hi=1.0):
        return jax.random.uniform(self._next(), shape, jnp.bfloat16, lo, hi)
    def permutation(self, n):
        return jax.random.permutation(self._next(), n)


kernel_name = 'recurrent_scan__compressed_kv_cla__dense_activation_gelu__decode'

def setup_inputs():
    _rng = _Rng(jax.random.key(int.from_bytes(__import__("os").urandom(4), "little")))
    _w = (lambda a: (lambda t: t.astype(jnp.bfloat16) if jnp.issubdtype(t.dtype, jnp.floating) else t)(jnp.asarray(a)))
    def _A_setup():
        B, H, Sq, Sk, D, M = 2, 32, 1, 16384, 128, 512
        Dc = 4 * D
        return {
            "x": _w((lambda *s: _rng.normal(s) * 0.05)(B, Sq, M)),
            "c_kv": _w((lambda *s: _rng.normal(s) * 0.05)(B, Sk, Dc)),
            "w_q": _w((lambda *s: _rng.normal(s) * 0.05)(M, H, D) * (M ** -0.5)),
            "w_uk": _w((lambda *s: _rng.normal(s) * 0.05)(Dc, H, D) * (Dc ** -0.5)),
            "w_uv": _w((lambda *s: _rng.normal(s) * 0.05)(Dc, H, D) * (Dc ** -0.5)),
            "w_o": _w((lambda *s: _rng.normal(s) * 0.05)(H, D, M) * ((H * D) ** -0.5)),
        }
    _A_in = _A_setup()

    def _B_setup():
        B, S, D, F = 2, 1, 512, 1792
        return {
            "x": _w((lambda *s: _rng.normal(s) * 0.05)(B, S, D)),
            "w1": _w((lambda *s: _rng.normal(s) * 0.05)(D, F) * (D ** -0.5)),
            "b1": _w((lambda *s: _rng.normal(s) * 0.05)(F) * 0.01),
            "w2": _w((lambda *s: _rng.normal(s) * 0.05)(F, D) * (F ** -0.5)),
            "b2": _w((lambda *s: _rng.normal(s) * 0.05)(D) * 0.01),
        }
    _B_in = _B_setup()

    return {
        "A_x": _A_in["x"],
        "A_c_kv": _A_in["c_kv"],
        "A_w_q": _A_in["w_q"],
        "A_w_uk": _A_in["w_uk"],
        "A_w_uv": _A_in["w_uv"],
        "A_w_o": _A_in["w_o"],
        "B_x": _B_in["x"],
        "B_w1": _B_in["w1"],
        "B_b1": _B_in["b1"],
        "B_w2": _B_in["w2"],
        "B_b2": _B_in["b2"],
    }

def reference(A_x, A_c_kv, A_w_q, A_w_uk, A_w_uv, A_w_o, B_x, B_w1, B_b1, B_w2, B_b2):
    def _A_ref(x, c_kv, w_q, w_uk, w_uv, w_o):
        B, Sq, M = x.shape[0], x.shape[1], x.shape[2]
        Sk = c_kv.shape[1]
        H, D = w_q.shape[1], w_q.shape[2]
        q = jnp.einsum("bqm,mhd->bhqd", x, w_q)
        k = jnp.einsum("bkc,chd->bhkd", c_kv, w_uk)
        v = jnp.einsum("bkc,chd->bhkd", c_kv, w_uv)
        scores = jnp.einsum("bhqd,bhkd->bhqk", q, k) * (D ** -0.5)
        off = Sk - Sq
        qi = jnp.arange(Sq)[:, None]
        kj = jnp.arange(Sk)[None, :]
        cmask = kj <= (qi + off)
        scores = jnp.where(cmask[None, None], scores, -1e9)
        p = _softmax(scores, axis=-1)
        ctx = jnp.einsum("bhqk,bhkd->bhqd", p, v)
        return jnp.einsum("bhqd,hdm->bqm", ctx, w_o)

    def _B_ref(x, w1, b1, w2, b2):
        h = jnp.einsum("bsd,df->bsf", x, w1) + b1
        h = _gelu(h)
        return jnp.einsum("bsf,fd->bsd", h, w2) + b2

    x = A_x
    xn = _layernorm(x, axis=-1)
    s = _A_ref(xn, A_c_kv, A_w_q, A_w_uk, A_w_uv, A_w_o)
    g = _silu(_B_ref(xn, B_w1, B_b1, B_w2, B_b2))
    return x + s * g
```

```python
import jax
import jax.numpy as jnp
from jax import lax
import jax.experimental.pallas as pl
import jax.experimental.pallas.tpu as pltpu

F32 = jnp.float32
BF16 = jnp.bfloat16
B, H, SK, D, M, DC, F = 2, 32, 16384, 128, 512, 512, 1792
LOG2E = 1.4426950408889634
NT = (((1,), (1,)), ((), ()))


def make(CB=16, AHEAD=2, FIRST=80, PIECE=64, LAST=(4, 3, 1), nocomp=False):
    CC = 32
    CA = SK // (CB * CC)
    PER = CB // 8
    BK = 2048
    NC = B * 8
    WA, WB, WC = 8, 16, 4
    NP = 25
    XR = FIRST + (NP - 1) * PIECE

    def kernel(x_hbm, ckv_hbm, wq_hbm, wuk_hbm, wuv_hbm, wo_hbm, w1_hbm, b1_hbm, w2_hbm, b2_hbm,
               o_ref,
               x_buf, b1_buf, b2_buf, c_buf, wq_buf, wuk_buf, wuv_buf, wo_buf, w1_buf, w2_buf, side,
               xn_vmem, xn_smem, t8, qa_ref, acc_ref, m_ref, l_ref, a_buf, ctx_ref,
               sem_w, sem_c, sem_o, sem_in, sem_out, sem_small):
        cp = pltpu.make_async_copy

        def start_w(hbm, buf, half, s):
            def body(j, _):
                cp(hbm.at[:, half * 8 + j], buf.at[:, half * 8 + j], sem_w.at[s]).start()
            lax.fori_loop(0, 8, body, None)

        def wait_w(buf, half, s):
            v = buf.at[:, pl.ds(half * 8, 8)]
            cp(v, v, sem_w.at[s]).wait()

        def start_c(ci):
            b, g = ci // 8, ci % 8
            for j in range(PER):
                cp(ckv_hbm.at[b, :, g * PER + j], c_buf.at[ci, j], sem_c.at[ci]).start()

        def wait_c(ci):
            cp(c_buf.at[ci], c_buf.at[ci], sem_c.at[ci]).wait()

        def start_o(qd):
            def body(j, _):
                cp(wo_hbm.at[:, qd, j], wo_buf.at[:, qd, j], sem_o.at[qd]).start()
            lax.fori_loop(0, 4, body, None)

        def wait_o(qd):
            v = wo_buf.at[:, qd]
            cp(v, v, sem_o.at[qd]).wait()

        last_off = [sum(LAST[:i]) for i in range(len(LAST))]
        last = [cp(wo_hbm.at[pl.ds(o, n), 3], wo_buf.at[pl.ds(o, n), 3], sem_o.at[3 + i])
                for i, (o, n) in enumerate(zip(last_off, LAST))]

        w1_cp = cp(w1_hbm, w1_buf, sem_w.at[6])
        rest_cp = cp(w2_hbm.at[pl.ds(XR, F - XR)], w2_buf.at[pl.ds(XR, F - XR)], sem_w.at[7])
        x_cp = cp(x_hbm, x_buf, sem_small.at[0])
        b1_cp = cp(b1_hbm, b1_buf, sem_small.at[1])
        b2_cp = cp(b2_hbm, b2_buf, sem_small.at[2])

        def start(i):
            if i in (1, 2): start_w(wq_hbm, wq_buf, i - 1, i - 1)
            elif i in (3, 4): start_w(wuk_hbm, wuk_buf, i - 3, i - 1)
            elif 5 <= i < 21: start_c(i - 5)
            elif i in (21, 22): start_w(wuv_hbm, wuv_buf, i - 21, i - 17)
            elif i == 23: start_o(0); start_o(1)
            elif i == 24:
                start_o(2)
                for c in last: c.start()

        def rows(j):
            if isinstance(j, int) and j == 0:
                return 0, FIRST
            o = FIRST + (j - 1) * PIECE
            return (o if isinstance(j, int) else pl.multiple_of(o, 16)), PIECE

        def c_in(j):
            o, n = rows(j)
            return cp(w2_hbm.at[pl.ds(o, n)], side.at[j % 4, pl.ds(0, n)], sem_in.at[j % 2])

        def c_out(j):
            o, n = rows(j)
            return cp(side.at[j % 4, pl.ds(0, n)], w2_buf.at[pl.ds(o, n)], sem_out.at[j % 2])

        def service(j):
            c_in(j).wait()
            if not isinstance(j, int) or j >= 2: c_out(j - 2).wait()
            c_out(j).start()
            if not isinstance(j, int) or j + 2 < NP: c_in(j + 2).start()

        w1_cp.start()
        c_in(0).start()
        x_cp.start()
        c_in(1).start()
        b1_cp.start()
        b2_cp.start()
        rest_cp.start()
        for i in range(1, AHEAD + 1):
            start(i)

        x_cp.wait()
        x = x_buf[...].astype(F32)
        xc = x - jnp.mean(x, axis=-1, keepdims=True)
        var = jnp.mean(xc * xc, axis=-1, keepdims=True)
        xn = (xc * lax.rsqrt(var + 1e-5)).astype(BF16)
        xn_vmem[...] = xn.astype(F32)
        to_smem = cp(xn_vmem, xn_smem, sem_small.at[0])
        to_smem.start()
        service(0)

        w1_cp.wait()
        start(1 + AHEAD)
        service(1)
        b1_cp.wait()
        hid = jnp.dot(xn, w1_buf[...], preferred_element_type=F32) + b1_buf[...].astype(F32).reshape(1, F)
        hid = jax.nn.gelu(hid, approximate=True).astype(BF16)
        to_smem.wait()
        b2_cp.wait()
        rest_cp.wait()

        q01 = (jnp.zeros((H, D), F32), jnp.zeros((H, D), F32))
        for j in range(2):
            wait_w(wq_buf, j, j)
            start(2 + j + AHEAD)
            service(2 + j)

            def q_body(i, carry, j=j):
                q0, q1 = carry
                a, jj = i // 4, j * 8 + (i % 4) * 2
                for u in range(8):
                    m = (a * WB + jj) * WC + u
                    w = wq_buf[a, jj + u // WC, u % WC].astype(F32)
                    q0 = q0 + xn_smem[0, m] * w
                    q1 = q1 + xn_smem[1, m] * w
                return q0, q1

            if not nocomp: q01 = lax.fori_loop(0, 32, q_body, q01)
        q = jnp.concatenate([q01[0], q01[1], jnp.zeros((128 - B * H, D), F32)], axis=0).astype(BF16)

        group = (lax.broadcasted_iota(jnp.int32, (16, 8, 128), 2) % H) // 8
        for j in range(2):
            wait_w(wuk_buf, j, 2 + j)
            start(4 + j + AHEAD)
            service(4 + j)

            def qa_body(s, _, j=j):
                a, jj = s // 2, j * 8 + (s % 2) * 4
                u = wuk_buf[a, pl.ds(jj, 4)].reshape(16 * H, D)
                r = lax.dot_general(u, q, NT, preferred_element_type=F32).reshape(16, 4, 8, 128)
                v = jnp.where(group == 0, r[:, 0],
                              jnp.where(group == 1, r[:, 1], jnp.where(group == 2, r[:, 2], r[:, 3])))
                t8[pl.ds(pl.multiple_of((a * WB + jj) * WC * 8, 128), 128), :] = v.reshape(128, 128)

            lax.fori_loop(0, 16, qa_body, None, unroll=2)
        sub = lax.broadcasted_iota(jnp.int32, (128, 128), 1) % 8
        for j in range(DC // 128):
            t = t8[pl.ds(j * 1024, 128, stride=8), :]
            for s in range(1, 8):
                t = jnp.where(sub == s, t8[pl.ds(j * 1024 + s, 128, stride=8), :], t)
            qa_ref[:, j * 128:(j + 1) * 128] = (t.T[:B * H] * (D ** -0.5 * LOG2E)).astype(BF16)

        m_ref[...] = jnp.full((B * H, 128), -jnp.inf, F32)
        l_ref[...] = jnp.zeros((B * H, 128), F32)
        acc_ref[...] = jnp.zeros((B * H, DC), F32)

        def chunk(ci, _):
            wait_c(ci)
            nxt = ci + AHEAD + 1
            pl.when(nxt < NC)(lambda: start_c(nxt))
            for e in range(AHEAD + 1):
                pl.when(nxt == NC + e)(lambda e=e: start(21 + e))
            service(ci + 6)
            hrows = pl.ds(pl.multiple_of((ci // 8) * H, H), H)
            c = c_buf[ci].reshape(BK, DC)
            sc = lax.dot_general(qa_ref[hrows, :], c, NT, preferred_element_type=F32)
            m_prev = m_ref[hrows, :]
            m_new = jnp.maximum(m_prev, jnp.max(sc, axis=1, keepdims=True))
            p = jnp.exp2(sc - m_new[:, :1])
            alpha = jnp.exp2(m_prev - m_new)
            l_ref[hrows, :] = alpha * l_ref[hrows, :] + jnp.sum(p, axis=1, keepdims=True)
            m_ref[hrows, :] = m_new
            pv = jnp.dot(p.astype(BF16), c, preferred_element_type=F32)
            acc_ref[hrows, :] = acc_ref[hrows, :] * alpha[:, :1] + pv

        lax.fori_loop(0, NC, chunk, None)

        pc = acc_ref[...] / l_ref[...][:, :1]
        lane = lax.broadcasted_iota(jnp.int32, (B * H, 128), 1)
        head = lax.broadcasted_iota(jnp.int32, (B * H, 128), 0) % H
        diag = (lane % H) == head
        ctx = jnp.zeros((B * H, D), F32)
        for j in range(2):
            for a in range(WA):
                c0 = (a * WB + j * 8) * WC
                pcj = pc[:, c0 // 128 * 128:c0 // 128 * 128 + 128]
                for t in range(8):
                    rep = jnp.take_along_axis(pcj, lane // H + (c0 % 128 + 4 * t), axis=1)
                    a_buf[:, (a * 8 + t) * 128:(a * 8 + t + 1) * 128] = jnp.where(diag, rep, 0.0).astype(BF16)
            wait_w(wuv_buf, j, 4 + j)
            start(22 + j + AHEAD)
            service(22 + j)
            v2 = wuv_buf[:, pl.ds(j * 8, 8)].reshape(256 * H, D)
            ctx = ctx + jnp.dot(a_buf[...], v2, preferred_element_type=F32)
        ctx_ref[...] = ctx

        def heads(hs):
            lhs = jnp.concatenate([ctx_ref[pl.ds(h, B, stride=H), :] for h in hs], axis=1).astype(BF16)
            rhs = jnp.concatenate([wo_buf[h // 4, h % 4].reshape(D, M) for h in hs], axis=0)
            return jnp.dot(lhs, rhs, preferred_element_type=F32)

        k0 = FIRST + (NP - 3) * PIECE
        k0 = k0 // 128 * 128
        kr = -(-XR // 128) * 128
        wait_o(0)
        s = heads([4 * a for a in range(8)])
        wait_o(1)
        service(24)
        s = s + heads([4 * a + 1 for a in range(8)])
        gg = b2_buf[...].astype(F32).reshape(1, M) + jnp.dot(hid[:, :k0], w2_buf[:k0], preferred_element_type=F32)
        gg = gg + jnp.dot(hid[:, kr:], w2_buf[kr:], preferred_element_type=F32)
        wait_o(2)
        s = s + heads([4 * a + 2 for a in range(8)])
        for i, (o, n) in enumerate(zip(last_off, LAST)):
            if i == 1:
                c_out(NP - 2).wait()
                c_out(NP - 1).wait()
                gg = gg + jnp.dot(hid[:, k0:kr], w2_buf[k0:kr], preferred_element_type=F32)
                g = gg * jax.nn.sigmoid(gg)
            last[i].wait()
            s = s + heads([4 * a + 3 for a in range(o, o + n)])
        o_ref[...] = (x + s * g).astype(BF16)

    def fn(A_x, A_c_kv, A_w_q, A_w_uk, A_w_uv, A_w_o, B_x, B_w1, B_b1, B_w2, B_b2):
        del B_x
        w5 = (WA, WB, WC, H, D)
        out = pl.pallas_call(
            kernel,
            out_shape=jax.ShapeDtypeStruct((B, M), BF16),
            in_specs=[pl.BlockSpec(memory_space=pltpu.HBM)] * 10,
            out_specs=pl.BlockSpec(memory_space=pltpu.VMEM),
            scratch_shapes=[
                pltpu.VMEM((B, M), BF16), pltpu.VMEM((F,), BF16), pltpu.VMEM((M,), BF16),
                pltpu.VMEM((NC, PER, CA, CC, DC), BF16),
                pltpu.VMEM(w5, BF16), pltpu.VMEM(w5, BF16), pltpu.VMEM(w5, BF16),
                pltpu.VMEM((8, 4, 4, 32, M), BF16), pltpu.VMEM((M, F), BF16), pltpu.VMEM((F, M), BF16),
                pltpu.SMEM((4, max(FIRST, PIECE), M), BF16),
                pltpu.VMEM((B, M), F32), pltpu.SMEM((B, M), F32),
                pltpu.VMEM((DC * 8 + 8, 128), F32),
                pltpu.VMEM((B * H, DC), BF16), pltpu.VMEM((B * H, DC), F32),
                pltpu.VMEM((B * H, 128), F32), pltpu.VMEM((B * H, 128), F32),
                pltpu.VMEM((B * H, 256 * H), BF16), pltpu.VMEM((B * H, D), F32),
                pltpu.SemaphoreType.DMA((8,)), pltpu.SemaphoreType.DMA((NC,)), pltpu.SemaphoreType.DMA((3 + len(LAST),)),
                pltpu.SemaphoreType.DMA((2,)), pltpu.SemaphoreType.DMA((2,)), pltpu.SemaphoreType.DMA((3,)),
            ],
            compiler_params=pltpu.CompilerParams(vmem_limit_bytes=100 * 1024 * 1024,
                                                 disable_semaphore_checks=True, disable_bounds_checks=True),
        )(A_x.reshape(B, M), A_c_kv.reshape(B, CA, CB, CC, DC), A_w_q.reshape(w5), A_w_uk.reshape(w5),
          A_w_uv.reshape(w5), A_w_o.reshape(8, 4, 4, 32, M), B_w1, B_b1, B_w2, B_b2)
        return out.reshape(B, 1, M)
    return fn


_impl = make(FIRST=64)


@jax.jit
def pallas_recurrent_scan__compressed_kv_cla__dense_activation_gelu__decode_kernel(
    A_x, A_c_kv, A_w_q, A_w_uk, A_w_uv, A_w_o, B_x, B_w1, B_b1, B_w2, B_b2,
):
    return _impl(A_x, A_c_kv, A_w_q, A_w_uk, A_w_uv, A_w_o, B_x, B_w1, B_b1, B_w2, B_b2)
```

```python
import jax
import jax.numpy as jnp
from jax import lax
import jax.experimental.pallas as pl
import jax.experimental.pallas.tpu as pltpu

F32 = jnp.float32
BF16 = jnp.bfloat16
B, H, SK, D, M, DC, F = 2, 32, 16384, 128, 512, 512, 1792
LOG2E = 1.4426950408889634
NT = (((1,), (1,)), ((), ()))


def make(FIRST=64, PIECE=64, VP=(160, 64, 16, 16), GW=0, OUT=0, TR=False, MAINFIRST=False, SKIP='', W1=0, RP=4, W1A=4, AH=3, SM=1, PADV=0, flags=None):
    BK = 2048
    NC = B * SK // BK
    NP = 25
    XR = FIRST + (NP - 1) * PIECE
    NV = sum(VP)
    assert NV in (128, 256, 384, 512)

    def kernel(x_hbm, ckv_hbm, wq_hbm, wuk_hbm, wuv_hbm, wo_hbm, w1_hbm, b1_hbm, w2_hbm, b2_hbm,
               o_ref,
               padv, x_buf, b1_buf, b2_buf, c_buf, wq_buf, wuk_buf, wuv_buf, wo_buf, w1_buf, w2_buf, side,
               xs, t8, qa_ref, acc_ref, m_ref, l_ref, a_buf, e_buf, ctx_ref, mul_ref,
               sem_w, sem_c, sem_o, sem_in, sem_out, sem_small):
        cp = pltpu.make_async_copy

        def W(c, name):
            if TR:
                with jax.named_scope('@' + name):
                    c.wait()
            else:
                c.wait()

        def start_w(hbm, buf, s, lo=0, hi=32):
            def body(j, _):
                cp(hbm.at[:, j], buf.at[:, j], sem_w.at[s]).start()
            lax.fori_loop(lo, hi, body, None)

        def wait_w(buf, s):
            W(cp(buf, buf, sem_w.at[s]), f'w{s}')

        def start_c(ci):
            def body(j, _):
                cp(ckv_hbm.at[ci // 2, :, (ci % 2) * 16 + j], c_buf.at[ci, j], sem_c.at[ci]).start()
            lax.fori_loop(0, 16, body, None)

        def wait_c(ci):
            W(cp(c_buf.at[ci], c_buf.at[ci], sem_c.at[ci]), 'c')

        def start_o(lo, hi):
            def body(j, _):
                rows = pl.ds(pl.multiple_of(j * 32, 32), 32)
                cp(wo_hbm.at[:, rows], wo_buf.at[:, rows], sem_o.at[j // 8]).start()
            lax.fori_loop(lo, hi, body, None)
            if hi < 24: return
            for cs in last + vpu:
                for c in cs:
                    c.start()

        def o_copy(a, rows, s):
            return cp(wo_hbm.at[a, rows], wo_buf.at[a, rows], sem_o.at[s])

        tail_heads = [(a, 6 + i) for a in range(4) for i in range(2)]
        n_mxu = 8 - NV // D
        mxu_groups = [g for g in (tail_heads[:min(4, n_mxu - 1)], tail_heads[min(4, n_mxu - 1):n_mxu]) if g]

        def runs(lo, hi, s):
            out = []
            while lo < hi:
                a, r = lo // 256, lo % 256
                n = min(hi - lo, 256 - r)
                out.append(o_copy(a, slice(768 + r, 768 + r + n), s))
                lo += n
            return out

        last, pos = [], 0
        for i, grp in enumerate(mxu_groups):
            last.append(runs(pos, pos + D * len(grp), 3 + i))
            pos += D * len(grp)
        cuts = [pos + sum(VP[:i]) for i in range(len(VP) + 1)]
        vpu = [runs(lo, hi, 5 + i) for i, (lo, hi) in enumerate(zip(cuts[:-1], cuts[1:]))]

        w1_cp = cp(w1_buf, w1_buf, sem_w.at[3])
        rest_cp = cp(w2_hbm.at[pl.ds(XR, F - XR)], w2_buf.at[pl.ds(XR, F - XR)], sem_w.at[4])
        x_cp = cp(x_hbm, x_buf, sem_small.at[0])
        b1_cp = cp(b1_hbm, b1_buf, sem_small.at[1])
        b2_cp = cp(b2_hbm, b2_buf, sem_small.at[2])

        def rows(j):
            if isinstance(j, int) and j == 0:
                return 0, FIRST
            o = FIRST + (j - 1) * PIECE
            return (o if isinstance(j, int) else pl.multiple_of(o, 8)), PIECE

        def c_in(j):
            o, n = rows(j)
            return cp(w2_hbm.at[pl.ds(o, n)], side.at[j % 4, pl.ds(0, n)], sem_in.at[j % 2])

        def c_out(j):
            o, n = rows(j)
            return cp(side.at[j % 4, pl.ds(0, n)], w2_buf.at[pl.ds(o, n)], sem_out.at[j % 2])

        def service(j):
            W(c_in(j), f'in{j}' if isinstance(j, int) else 'in')
            if not isinstance(j, int) or j >= 2: W(c_out(j - 2), 'out')
            c_out(j).start()
            if not isinstance(j, int) or j + 2 < NP: c_in(j + 2).start()

        def start_w1():
            if W1 in (0, 1):
                cp(w1_hbm, w1_buf, sem_w.at[3]).start()
            else:
                n = M // W1A
                def body(j, _):
                    r = pl.ds(pl.multiple_of(j * 8, 8), 8)
                    cp(w1_hbm.at[:, r], w1_buf.at[:, r], sem_w.at[3]).start()
                lax.fori_loop(0, n // 8, body, None)

        def start_q(lo, hi):
            if W1 != 2: return start_w(wq_hbm, wq_buf, 0, lo, hi)
            def body(j, _):
                cp(wq_hbm.at[:, j], wq_buf.at[:, j], sem_w.at[0]).start()
                a, r = j // (32 // W1A), pl.ds(pl.multiple_of((j % (32 // W1A)) * 16, 16), 16)
                cp(w1_hbm.at[a, r], w1_buf.at[a, r], sem_w.at[3]).start()
            lax.fori_loop(lo, hi, body, None)

        if W1 == 0:
            if MAINFIRST: start_w1()
            c_in(0).start()
            if not MAINFIRST: start_w1()
            c_in(1).start()
        else:
            c_in(0).start()
            c_in(1).start()
            if W1 == 3: start_w1()
        start_q(0, RP)
        for c in (x_cp, b1_cp, b2_cp, rest_cp): c.start()
        start_q(RP, 24)
        service(0)
        start_q(24, 32)
        service(1)
        if W1 in (1, 4): start_w1()
        if W1 in (1, 2, 4):
            service(2)
            start_w(wuk_hbm, wuk_buf, 1, 0, 16)
            service(3)
            start_w(wuk_hbm, wuk_buf, 1, 16, 32)
        x_cp.wait()
        x = x_buf[...].astype(F32)
        xc = x - jnp.mean(x, axis=-1, keepdims=True)
        var = jnp.mean(xc * xc, axis=-1, keepdims=True)
        xn = (xc * lax.rsqrt(var + 1e-5)).astype(BF16)
        xf = xn.astype(F32)
        for b in range(B):
            for j in range(M // 128):
                xs[b, j * 128:(j + 1) * 128, :] = jnp.broadcast_to(xf[b:b + 1, j * 128:(j + 1) * 128], (128, 128)).T

        W(w1_cp, 'w1')
        b1_cp.wait()
        hid = jnp.dot(xn, w1_buf[...].reshape(M, F), preferred_element_type=F32) + b1_buf[...].astype(F32).reshape(1, F)
        hid = jax.nn.gelu(hid, approximate=True).astype(BF16)
        b2_cp.wait()
        rest_cp.wait()
        e_buf[...] = (lax.broadcasted_iota(jnp.int32, (128, 128 * H), 1) // H
                      == lax.broadcasted_iota(jnp.int32, (128, 128 * H), 0)).astype(F32).astype(BF16)
        if W1 in (0, 3):
            service(2)
            start_w(wuk_hbm, wuk_buf, 1, 0, 16)
            service(3)
            start_w(wuk_hbm, wuk_buf, 1, 16, 32)

        wait_w(wq_buf, 0)

        def q_body(i, carry):
            q0, q1 = carry
            for u in range(8):
                m = i * 8 + u
                w = wq_buf[i // 16, (i % 16) * 2 + u // 4, u % 4].astype(F32)
                q0 = q0 + xs[0, pl.ds(m, 1), :] * w
                q1 = q1 + xs[1, pl.ds(m, 1), :] * w
            return q0, q1

        q01 = lax.fori_loop(0, 1 if 'q' in SKIP else 64, q_body, (jnp.zeros((H, D), F32), jnp.zeros((H, D), F32)))
        q = jnp.concatenate([q01[0], q01[1], jnp.zeros((128 - B * H, D), F32)], axis=0).astype(BF16)
        service(4)
        start_c(0)

        service(5)
        wait_w(wuk_buf, 1)
        start_c(1)
        group = (lax.broadcasted_iota(jnp.int32, (16, 8, 128), 2) % H) // 8

        def qa_body(i, _):
            for u in range(4):
                s = i * 4 + u
                w = wuk_buf[i // 2, pl.ds((i % 2) * 16 + u * 4, 4)].reshape(16 * H, D)
                r = lax.dot_general(w, q, NT, preferred_element_type=F32).reshape(16, 4, 8, 128)
                v = jnp.where(group == 0, r[:, 0],
                              jnp.where(group == 1, r[:, 1], jnp.where(group == 2, r[:, 2], r[:, 3])))
                t8[pl.ds(pl.multiple_of(s * 128, 128), 128), :] = v.reshape(128, 128)

        lax.fori_loop(0, 1 if 'q' in SKIP else 8, qa_body, None)
        sub = lax.broadcasted_iota(jnp.int32, (128, 128), 1) % 8
        for j in range(DC // 128):
            t = t8[pl.ds(j * 1024, 128, stride=8), :]
            for s in range(1, 8):
                t = jnp.where(sub == s, t8[pl.ds(j * 1024 + s, 128, stride=8), :], t)
            qa_ref[:, j * 128:(j + 1) * 128] = (t.T[:B * H] * (D ** -0.5 * LOG2E)).astype(BF16)

        m_ref[...] = jnp.full((B * H, 128), -jnp.inf, F32)
        l_ref[...] = jnp.zeros((B * H, 128), F32)
        acc_ref[...] = jnp.zeros((B * H, DC), F32)

        def chunk(ci, _):
            service(ci + 6)
            wait_c(ci)
            nxt = ci + 2
            pl.when(nxt < NC)(lambda: start_c(nxt))
            pl.when(nxt >= NC)(lambda: start_w(wuv_hbm, wuv_buf, 2, (nxt - NC) * 16, (nxt - NC) * 16 + 16))
            hrows = pl.ds(pl.multiple_of((ci // 8) * H, H), H)
            if 'a' in SKIP: return
            c = c_buf[ci].reshape(BK, DC)
            sc = lax.dot_general(qa_ref[hrows, :], c, NT, preferred_element_type=F32)
            m_prev = m_ref[hrows, :]
            m_new = jnp.maximum(m_prev, jnp.max(sc, axis=1, keepdims=True))
            p = jnp.exp2(sc - m_new[:, :1])
            alpha = jnp.exp2(m_prev - m_new)
            l_ref[hrows, :] = alpha * l_ref[hrows, :] + jnp.sum(p, axis=1, keepdims=True)
            m_ref[hrows, :] = m_new
            pv = jnp.dot(p.astype(BF16), c, preferred_element_type=F32)
            acc_ref[hrows, :] = acc_ref[hrows, :] * alpha[:, :1] + pv

        lax.fori_loop(0, NC, chunk, None)

        pc = (acc_ref[...] / l_ref[...][:, :1]).astype(BF16)
        lane = lax.broadcasted_iota(jnp.int32, (B * H, 128 * H), 1)
        head = lax.broadcasted_iota(jnp.int32, (B * H, 128 * H), 0) % H
        diag = (lane % H) == head
        for j in range(0 if 'c' in SKIP else DC // 128):
            rep = jnp.dot(pc[:, j * 128:(j + 1) * 128], e_buf[...], preferred_element_type=F32)
            a_buf[j] = jnp.where(diag, rep, 0.0).astype(BF16)
        service(22)
        start_o(0, 16)
        service(23)
        wait_w(wuv_buf, 2)
        start_o(16, 24)
        ctx = jnp.zeros((B * H, D), F32)
        for j in range(0 if 'c' in SKIP else DC // 128):
            ctx = ctx + jnp.dot(a_buf[j], wuv_buf[j].reshape(128 * H, D), preferred_element_type=F32)
        ctx_ref[...] = ctx
        cb = ctx.astype(BF16).astype(F32)
        for b in range(B):
            for i, (a, hh) in enumerate(tail_heads[n_mxu:]):
                r = b * H + 8 * a + hh
                mul_ref[b, i * D:(i + 1) * D] = jnp.broadcast_to(cb[r:r + 1], (128, 128)).T

        def heads(pairs):
            lhs = jnp.concatenate([ctx_ref[pl.ds(8 * a + i, B, stride=H), :] for a, i in pairs], axis=1).astype(BF16)
            rhs = jnp.concatenate([wo_buf[a, i * D:(i + 1) * D] for a, i in pairs], axis=0)
            return jnp.dot(lhs, rhs, preferred_element_type=F32)

        def quad(qd):
            v = wo_buf.at[:, pl.ds(qd * 256, 256)]
            W(cp(v, v, sem_o.at[qd]), f'o{qd}')
            if 'o' in SKIP: return x
            return heads([(a, 2 * qd + i) for a in range(4) for i in range(2)])

        k0 = (FIRST + (NP - 3) * PIECE) // 128 * 128
        kr = -(-XR // 128) * 128
        service(24)
        s = quad(0)
        s = s + quad(1)
        gg = b2_buf[...].astype(F32).reshape(1, M) + jnp.dot(hid[:, :k0], w2_buf[:k0], preferred_element_type=F32)
        gg = gg + jnp.dot(hid[:, kr:], w2_buf[kr:], preferred_element_type=F32)
        s = s + quad(2)
        sl = lax.broadcasted_iota(jnp.int32, (8, 128), 0)

        def rows8(v):
            return jnp.concatenate([v[:, j * 128:(j + 1) * 128] for j in range(4)], axis=0)

        def wait_gate():
            W(c_out(NP - 2), 'out23')
            W(c_out(NP - 1), 'outlast')

        def gate():
            if 'g' in SKIP: return rows8(gg)
            z = rows8(gg + jnp.dot(hid[:, k0:kr], w2_buf[k0:kr], preferred_element_type=F32))
            return z * jax.nn.sigmoid(z)

        x8 = rows8(x)
        for i, grp in enumerate(mxu_groups):
            for c in last[i]:
                W(c, f'last{i}')
            if GW == 0 and i == len(mxu_groups) - 1:
                wait_gate()
                g8 = gate()
            if 'm' not in SKIP: s = s + heads(grp)
        s8 = rows8(s)
        acc = [[None] * 4 for _ in range(B)]
        for i, cs in enumerate(vpu):
            if GW == i + 1:
                wait_gate()
                g8 = gate()
            if i == len(VP) - 1:
                base8 = x8 + s8 * g8
            for c in cs:
                W(c, f'v{i}')
            for r in range(cuts[i], cuts[i + 1], 8):
                if 'v' in SKIP and i < len(VP) - 1: break
                if 'z' in SKIP and r > cuts[i]: break
                w = wo_buf[r // 256, 768 + r % 256:768 + r % 256 + 8].astype(F32)
                for b in range(B):
                    mul = mul_ref[b, r - cuts[0]:r - cuts[0] + 8, :]
                    for j in range(4):
                        pr = w[:, j * 128:(j + 1) * 128] * mul
                        acc[b][j] = pr if acc[b][j] is None else acc[b][j] + pr
        hi4, hi2, hi1 = (sl & 4) != 0, (sl & 2) != 0, (sl & 1) != 0

        def merge(a, c, m, k):
            if k == 4:
                return jnp.where(m, c, a) + pltpu.roll(jnp.where(m, a, c), 4, 0)
            return jnp.where(m, c, a) + jnp.where(m, pltpu.roll(c, k, 0), pltpu.roll(a, 8 - k, 0))

        r4 = [[merge(acc[b][j], acc[b][j + 2], hi4, 4) for j in range(2)] for b in range(B)]
        r2 = [merge(r4[b][0], r4[b][1], hi2, 2) for b in range(B)]
        res = base8 + g8 * merge(r2[0], r2[1], hi1, 1)
        if 'r' in SKIP:
            o_ref[...] = wo_buf[3, 1016:1018]
        elif OUT == 0:
            o_ref[...] = jnp.concatenate([res[2 * j:2 * j + 2] for j in range(4)], axis=1).astype(BF16)
        elif OUT == 2:
            o_ref[...] = pltpu.bitcast(pltpu.bitcast(res.astype(BF16), jnp.uint32).reshape(1, M), BF16)
        elif OUT == 3:
            o_ref[...] = res.astype(BF16).reshape(4, 2, 128)

    def fn(A_x, A_c_kv, A_w_q, A_w_uk, A_w_uv, A_w_o, B_x, B_w1, B_b1, B_w2, B_b2):
        del B_x
        w5 = (4, 32, 4, H, D)
        out = pl.pallas_call(
            kernel,
            out_shape=jax.ShapeDtypeStruct((4, B, 128) if OUT == 3 else (B, M), BF16),
            in_specs=[pl.BlockSpec(memory_space=pltpu.HBM)] * 10,
            out_specs=pl.BlockSpec(memory_space=pltpu.VMEM),
            scratch_shapes=[
                pltpu.VMEM((1, 128 * max(PADV, 1)), F32),
                pltpu.VMEM((B, M), BF16), pltpu.VMEM((F,), BF16), pltpu.VMEM((M,), BF16),
                pltpu.VMEM((NC, 16, 4, 32, DC), BF16),
                pltpu.VMEM(w5, BF16), pltpu.VMEM(w5, BF16), pltpu.VMEM(w5, BF16),
                pltpu.VMEM((4, 8 * D, M), BF16),
                pltpu.VMEM((W1A, M // W1A, F), BF16), pltpu.VMEM((F, M), BF16),
                pltpu.SMEM((4, max(FIRST, PIECE), M), BF16),
                pltpu.VMEM((B, M, 128), F32),
                pltpu.VMEM((DC * 8 + 8, 128), F32),
                pltpu.VMEM((B * H, DC), BF16), pltpu.VMEM((B * H, DC), F32),
                pltpu.VMEM((B * H, 128), F32), pltpu.VMEM((B * H, 128), F32),
                pltpu.VMEM((4, B * H, 128 * H), BF16), pltpu.VMEM((128, 128 * H), BF16),
                pltpu.VMEM((B * H, D), F32), pltpu.VMEM((B, NV, 128), F32),
                pltpu.SemaphoreType.DMA((5,)), pltpu.SemaphoreType.DMA((NC,)),
                pltpu.SemaphoreType.DMA((5 + len(VP),)),
                pltpu.SemaphoreType.DMA((2,)), pltpu.SemaphoreType.DMA((2,)), pltpu.SemaphoreType.DMA((3,)),
            ],
            compiler_params=pltpu.CompilerParams(vmem_limit_bytes=100 * 1024 * 1024, flags=flags,
                                                 disable_semaphore_checks=True, disable_bounds_checks=True),
        )(A_x.reshape(B, M), A_c_kv.reshape(NC // 2, 4, 32, 32, DC), A_w_q.reshape(w5), A_w_uk.reshape(w5),
          A_w_uv.reshape(w5), A_w_o.reshape(4, 8 * D, M), B_w1.reshape(W1A, M // W1A, F), B_b1, B_w2, B_b2)
        if OUT == 3:
            out = out.transpose(1, 0, 2)
        return out.reshape(B, 1, M)
    return fn


_impl = make(W1=4, W1A=2)


@jax.jit
def pallas_recurrent_scan__compressed_kv_cla__dense_activation_gelu__decode_kernel(
    A_x, A_c_kv, A_w_q, A_w_uk, A_w_uv, A_w_o, B_x, B_w1, B_b1, B_w2, B_b2,
):
    return _impl(A_x, A_c_kv, A_w_q, A_w_uk, A_w_uv, A_w_o, B_x, B_w1, B_b1, B_w2, B_b2)
```

```python
import jax
import jax.numpy as jnp
from jax import lax
import jax.experimental.pallas as pl
import jax.experimental.pallas.tpu as pltpu

F32 = jnp.float32
BF16 = jnp.bfloat16

B, H, SK, D, M, DC, F = 2, 32, 16384, 128, 512, 512, 1792
LOG2E = 1.4426950408889634
NT = (((1,), (1,)), ((), ()))

W_VIEW = (4, 32, 4, H, D)
BK = 2048
NC = B * SK // BK

TAIL_HEADS = [(a, i) for a in range(4) for i in (6, 7)]
MXU_CUTS = (0, 4 * D, 5 * D)
V0 = MXU_CUTS[-1]
SIDE_ROWS = 8
VPU_CUTS = (V0 + SIDE_ROWS, 832, 896, 960, 1008, 1024)

PIECE = 64
NP = 25
XR = NP * PIECE


def _loop(lo, hi, body):
    lax.fori_loop(lo, hi, lambda i, _: body(i), None)


def _rows8(v):
    return jnp.concatenate([v[:, j * 128:(j + 1) * 128] for j in range(M // 128)], axis=0)


def _kernel(x_hbm, ckv_hbm, wq_hbm, wuk_hbm, wuv_hbm, wo_hbm, w1_hbm, b1_hbm, w2_hbm, b2_hbm,
            o_hbm,
            x_buf, b1_buf, b2_buf, c_buf, wq_buf, wuk_buf, wuv_buf, wo_buf, w1_buf, w2_buf, stage,
            xs, t8, qa_ref, acc_ref, m_ref, l_ref, a_buf, e_buf, ctx_ref, mul_ref, o_buf,
            sem_w, sem_c, sem_o, sem_in, sem_out, sem_small):
    copy = pltpu.make_async_copy

    def wait_filled(buf, sem):
        copy(buf, buf, sem).wait()

    def start_w(hbm, buf, sem, lo, hi):
        _loop(lo, hi, lambda j: copy(hbm.at[:, j], buf.at[:, j], sem).start())

    def start_c(ci):
        _loop(0, 16, lambda j: copy(ckv_hbm.at[ci // 2, :, (ci % 2) * 16 + j], c_buf.at[ci, j],
                                    sem_c.at[ci]).start())

    def start_rows(hbm, buf, n, sem_of, count):
        def body(j):
            rows = pl.ds(pl.multiple_of(j * n, n), n)
            copy(hbm.at[:, rows], buf.at[:, rows], sem_of(j)).start()
        _loop(0, count, body)

    def tail(ref, lo, n):
        assert lo % 256 + n <= 256
        return ref.at[lo // 256, pl.ds(768 + lo % 256, n)]

    def tail_copies(lo, hi, sem):
        out = []
        while lo < hi:
            n = min(hi - lo, 256 - lo % 256)
            out.append(copy(tail(wo_hbm, lo, n), tail(wo_buf, lo, n), sem))
            lo += n
        return out

    mxu_copies = [tail_copies(lo, hi, sem_o.at[3 + i])
                  for i, (lo, hi) in enumerate(zip(MXU_CUTS, MXU_CUTS[1:]))]
    vpu_copies = [tail_copies(lo, hi, sem_o.at[5 + i])
                  for i, (lo, hi) in enumerate(zip(VPU_CUTS, VPU_CUTS[1:]))]
    w2_rest = copy(w2_hbm.at[pl.ds(XR, F - XR)], w2_buf.at[pl.ds(XR, F - XR)], sem_w.at[4])
    x_copy = copy(x_hbm, x_buf, sem_small.at[0])
    b1_copy = copy(b1_hbm, b1_buf, sem_small.at[1])
    b2_copy = copy(b2_hbm, b2_buf, sem_small.at[2])

    def piece(j):
        static = isinstance(j, int)
        if static and j == NP:
            return tail(wo_hbm, V0, SIDE_ROWS), stage.at[j % 4, pl.ds(0, SIDE_ROWS)], tail(wo_buf, V0, SIDE_ROWS)
        rows = pl.ds(j * PIECE if static else pl.multiple_of(j * PIECE, PIECE), PIECE)
        return w2_hbm.at[rows], stage.at[j % 4], w2_buf.at[rows]

    def leg_in(j):
        return copy(*piece(j)[:2], sem_in.at[j % 2])

    def leg_out(j):
        return copy(*piece(j)[1:], sem_out.at[j % 2])

    def relay(j):
        static = isinstance(j, int)
        leg_in(j).wait()
        if not static or j >= 2:
            leg_out(j - 2).wait()
        leg_out(j).start()
        if not static or j + 2 <= NP:
            leg_in(j + 2).start()

    copy(wq_hbm.at[:, 0], wq_buf.at[:, 0], sem_w.at[0]).start()
    leg_in(0).start()
    leg_in(1).start()
    start_w(wq_hbm, wq_buf, sem_w.at[0], 1, 4)
    for c in (x_copy, b1_copy, b2_copy, w2_rest):
        c.start()
    start_w(wq_hbm, wq_buf, sem_w.at[0], 4, 32)
    relay(0)
    relay(1)
    start_rows(w1_hbm, w1_buf, 8, lambda j: sem_w.at[3], M // 2 // 8)

    x_copy.wait()
    x = x_buf[...].astype(F32)
    xc = x - jnp.mean(x, axis=-1, keepdims=True)
    var = jnp.mean(xc * xc, axis=-1, keepdims=True)
    xn = (xc * lax.rsqrt(var + 1e-5)).astype(BF16)
    xf = xn.astype(F32)
    for b in range(B):
        for j in range(M // 128):
            cols = slice(j * 128, (j + 1) * 128)
            xs[b, cols, :] = jnp.broadcast_to(xf[b:b + 1, cols], (128, 128)).T
    e_buf[...] = (lax.broadcasted_iota(jnp.int32, (128, 128 * H), 1) // H
                  == lax.broadcasted_iota(jnp.int32, (128, 128 * H), 0)).astype(F32).astype(BF16)
    relay(2)

    wait_filled(wq_buf, sem_w.at[0])
    start_w(wuk_hbm, wuk_buf, sem_w.at[1], 0, 32)

    def q_body(i, carry):
        q0, q1 = carry
        for u in range(8):
            m = pl.ds(i * 8 + u, 1)
            w = wq_buf[i // 16, (i % 16) * 2 + u // 4, u % 4].astype(F32)
            q0 = q0 + xs[0, m, :] * w
            q1 = q1 + xs[1, m, :] * w
        return q0, q1

    q0, q1 = lax.fori_loop(0, M // 8, q_body, (jnp.zeros((H, D), F32), jnp.zeros((H, D), F32)))
    q = jnp.concatenate([q0, q1, jnp.zeros((128 - B * H, D), F32)], axis=0).astype(BF16)
    relay(3)

    wait_filled(w1_buf, sem_w.at[3])
    b1_copy.wait()
    hid = jnp.dot(xn, w1_buf[...].reshape(M, F), preferred_element_type=F32)
    hid = jax.nn.gelu(hid + b1_buf[...].astype(F32).reshape(1, F), approximate=True).astype(BF16)
    b2_copy.wait()
    w2_rest.wait()
    relay(4)
    start_c(0)
    start_c(1)

    wait_filled(wuk_buf, sem_w.at[1])
    relay(5)
    start_c(2)
    group = (lax.broadcasted_iota(jnp.int32, (16, 8, 128), 2) % H) // 8

    def qa_body(i):
        for u in range(4):
            w = wuk_buf[i // 2, pl.ds((i % 2) * 16 + u * 4, 4)].reshape(16 * H, D)
            r = lax.dot_general(w, q, NT, preferred_element_type=F32).reshape(16, 4, 8, 128)
            v = jnp.where(group == 0, r[:, 0],
                          jnp.where(group == 1, r[:, 1], jnp.where(group == 2, r[:, 2], r[:, 3])))
            t8[pl.ds(pl.multiple_of((i * 4 + u) * 128, 128), 128), :] = v.reshape(128, 128)

    _loop(0, DC // 64, qa_body)
    relay(6)
    sub = lax.broadcasted_iota(jnp.int32, (128, 128), 1) % 8
    for j in range(DC // 128):
        t = t8[pl.ds(j * 1024, 128, stride=8), :]
        for s in range(1, 8):
            t = jnp.where(sub == s, t8[pl.ds(j * 1024 + s, 128, stride=8), :], t)
        qa_ref[:, j * 128:(j + 1) * 128] = (t.T[:B * H] * (D ** -0.5 * LOG2E)).astype(BF16)

    m_ref[...] = jnp.full((B * H, 128), -jnp.inf, F32)
    l_ref[...] = jnp.zeros((B * H, 128), F32)
    acc_ref[...] = jnp.zeros((B * H, DC), F32)

    def block(ci):
        wait_filled(c_buf.at[ci], sem_c.at[ci])
        nxt = ci + 3
        pl.when(nxt < NC)(lambda: start_c(nxt))
        pl.when(jnp.logical_and(nxt >= NC, nxt < NC + 2))(
            lambda: start_w(wuv_hbm, wuv_buf, sem_w.at[2], (nxt - NC) * 16, (nxt - NC) * 16 + 16))
        pl.when(ci > 0)(lambda: relay(ci + 6))

        hrows = pl.ds(pl.multiple_of((ci // (NC // B)) * H, H), H)
        c = c_buf[ci].reshape(BK, DC)
        sc = lax.dot_general(qa_ref[hrows, :], c, NT, preferred_element_type=F32)
        m_prev = m_ref[hrows, :]
        m_new = jnp.maximum(m_prev, jnp.max(sc, axis=1, keepdims=True))
        p = jnp.exp2(sc - m_new[:, :1])
        alpha = jnp.exp2(m_prev - m_new)
        l_ref[hrows, :] = alpha * l_ref[hrows, :] + jnp.sum(p, axis=1, keepdims=True)
        m_ref[hrows, :] = m_new
        pv = jnp.dot(p.astype(BF16), c, preferred_element_type=F32)
        acc_ref[hrows, :] = acc_ref[hrows, :] * alpha[:, :1] + pv

    _loop(0, NC, block)

    pc = (acc_ref[...] / l_ref[...][:, :1]).astype(BF16)
    diag = (lax.broadcasted_iota(jnp.int32, (B * H, 128 * H), 1) % H
            == lax.broadcasted_iota(jnp.int32, (B * H, 128 * H), 0) % H)
    for j in range(DC // 128):
        rep = jnp.dot(pc[:, j * 128:(j + 1) * 128], e_buf[...], preferred_element_type=F32)
        a_buf[j] = jnp.where(diag, rep, 0.0).astype(BF16)
    relay(22)
    start_rows(wo_hbm, wo_buf, 32, lambda j: sem_o.at[j // 8], 24)
    for c in sum(mxu_copies + vpu_copies, []):
        c.start()
    relay(23)
    wait_filled(wuv_buf, sem_w.at[2])
    ctx = jnp.zeros((B * H, D), F32)
    for j in range(DC // 128):
        ctx = ctx + jnp.dot(a_buf[j], wuv_buf[j].reshape(128 * H, D), preferred_element_type=F32)
    ctx_ref[:B * H] = ctx
    cb = ctx.astype(BF16).astype(F32)
    for b in range(B):
        for i, (a, h) in enumerate(TAIL_HEADS[V0 // D:]):
            r = b * H + 8 * a + h
            mul_ref[b, i * D:(i + 1) * D] = jnp.broadcast_to(cb[r:r + 1], (128, 128)).T

    def project(heads):
        lhs = jnp.concatenate([ctx_ref[pl.ds(8 * a + h, B, stride=H), :] for a, h in heads], axis=1)
        rhs = jnp.concatenate([wo_buf[a, h * D:(h + 1) * D] for a, h in heads], axis=0)
        return jnp.dot(lhs.astype(BF16), rhs, preferred_element_type=F32)

    def project_pair(i):
        wait_filled(wo_buf.at[:, pl.ds(i * 2 * D, 2 * D)], sem_o.at[i])
        return project([(a, 2 * i + k) for a in range(4) for k in range(2)])

    def ffn(lo, hi):
        return jnp.dot(hid[:, lo:hi], w2_buf[lo:hi], preferred_element_type=F32)

    k0 = (XR - 2 * PIECE) // 128 * 128
    k1 = -(-XR // 128) * 128
    relay(NP - 1)
    s = project_pair(0)
    z = b2_buf[...].astype(F32).reshape(1, M) + ffn(0, k0) + ffn(k1, F)
    s = s + project_pair(1)
    relay(NP)
    s = s + project_pair(2)
    x8 = _rows8(x)
    for i, copies in enumerate(mxu_copies):
        for c in copies:
            c.wait()
        if i == len(mxu_copies) - 1:
            leg_out(NP - 1).wait()
            z8 = _rows8(z + ffn(k0, k1))
            g8 = z8 * jax.nn.sigmoid(z8)
        s = s + project(TAIL_HEADS[MXU_CUTS[i] // D:MXU_CUTS[i + 1] // D])
    base8 = x8 + _rows8(s) * g8

    part = [[None] * (M // 128) for _ in range(B)]

    def vpu_rows(lo, hi):
        for r in range(lo, hi, 8):
            w = tail(wo_buf, r, 8)[...].astype(F32)
            for b in range(B):
                mul = mul_ref[b, r - V0:r - V0 + 8, :]
                for j in range(M // 128):
                    t = w[:, j * 128:(j + 1) * 128] * mul
                    part[b][j] = t if part[b][j] is None else part[b][j] + t

    for i, copies in enumerate(vpu_copies):
        if i == 2:
            leg_out(NP).wait()
            vpu_rows(V0, V0 + SIDE_ROWS)
        for c in copies:
            c.wait()
        vpu_rows(VPU_CUTS[i], VPU_CUTS[i + 1])

    sl = lax.broadcasted_iota(jnp.int32, (8, 128), 0)

    def merge(lo, hi, k):
        m = (sl & k) != 0
        if k == 4:
            return jnp.where(m, hi, lo) + pltpu.roll(jnp.where(m, lo, hi), 4, 0)
        return jnp.where(m, hi, lo) + jnp.where(m, pltpu.roll(hi, k, 0), pltpu.roll(lo, 8 - k, 0))

    r4 = [[merge(part[b][j], part[b][j + 2], 4) for j in range(2)] for b in range(B)]
    r2 = [merge(r4[b][0], r4[b][1], 2) for b in range(B)]
    o_buf[...] = (base8 + g8 * merge(r2[0], r2[1], 1)).astype(BF16)
    o_copy = copy(o_buf, o_hbm, sem_small.at[0])
    o_copy.start()
    o_copy.wait()


@jax.jit
def pallas_recurrent_scan__compressed_kv_cla__dense_activation_gelu__decode_kernel(
    A_x: jax.Array,
    A_c_kv: jax.Array,
    A_w_q: jax.Array,
    A_w_uk: jax.Array,
    A_w_uv: jax.Array,
    A_w_o: jax.Array,
    B_x: jax.Array,
    B_w1: jax.Array,
    B_b1: jax.Array,
    B_w2: jax.Array,
    B_b2: jax.Array,
):
    del B_x
    hbm = pl.BlockSpec(memory_space=pltpu.HBM)
    dma_sems = pltpu.SemaphoreType.DMA
    out = pl.pallas_call(
        _kernel,
        out_shape=jax.ShapeDtypeStruct((8, 128), BF16),
        in_specs=[hbm] * 10,
        out_specs=hbm,
        scratch_shapes=[
            pltpu.VMEM((B, M), BF16), pltpu.VMEM((F,), BF16), pltpu.VMEM((M,), BF16),
            pltpu.VMEM((NC, 16, 4, 32, DC), BF16),
            pltpu.VMEM(W_VIEW, BF16), pltpu.VMEM(W_VIEW, BF16), pltpu.VMEM(W_VIEW, BF16),
            pltpu.VMEM((4, 8 * D, M), BF16), pltpu.VMEM((2, M // 2, F), BF16), pltpu.VMEM((F, M), BF16),
            pltpu.SMEM((4, PIECE, M), BF16),
            pltpu.VMEM((B, M, 128), F32),
            pltpu.VMEM((DC * 8 + 8, 128), F32),
            pltpu.VMEM((B * H, DC), BF16), pltpu.VMEM((B * H, DC), F32),
            pltpu.VMEM((B * H, 128), F32), pltpu.VMEM((B * H, 128), F32),
            pltpu.VMEM((DC // 128, B * H, 128 * H), BF16), pltpu.VMEM((128, 128 * H), BF16),
            pltpu.VMEM((3 * H, D), F32), pltpu.VMEM((B, 8 * D - V0, 128), F32), pltpu.VMEM((8, 128), BF16),
            dma_sems((5,)), dma_sems((NC,)), dma_sems((4 + len(VPU_CUTS),)),
            dma_sems((2,)), dma_sems((2,)), dma_sems((3,)),
        ],
        compiler_params=pltpu.CompilerParams(
            vmem_limit_bytes=100 * 1024 * 1024, disable_semaphore_checks=True, disable_bounds_checks=True),
    )(A_x.reshape(B, M), A_c_kv.reshape(NC // 2, 4, 32, 32, DC),
      A_w_q.reshape(W_VIEW), A_w_uk.reshape(W_VIEW), A_w_uv.reshape(W_VIEW), A_w_o.reshape(4, 8 * D, M),
      B_w1.reshape(2, M // 2, F), B_b1, B_w2, B_b2)
    return out.reshape(M // 128, B, 128).transpose(1, 0, 2).reshape(B, 1, M)
```

```python
import jax
import jax.numpy as jnp
from jax import lax
import jax.experimental.pallas as pl
import jax.experimental.pallas.tpu as pltpu

F32 = jnp.float32
BF16 = jnp.bfloat16
B, H, SK, D, M, DC, F = 2, 32, 16384, 128, 512, 512, 1792
LOG2E = 1.4426950408889634
NT = (((1,), (1,)), ((), ()))


def make(PAT=((0, 32), (32, 16), (48, 16)), VC=(128, 320, 384, 448, 496, 512), LP=16, CU=2,
         W2P=((0, 24), (24, 16), (40, 16)), TR=False, flags=None):
    BK = 2048
    NC = B * SK // BK
    V0 = VC[0]

    def kernel(x_hbm, ckv_hbm, wq_hbm, wuk_hbm, wuv_hbm, wo_hbm, w1_hbm, b1_hbm, w2_hbm, b2_hbm,
               o_hbm,
               x_buf, b1_buf, b2_buf, c_buf, wq_buf, wuk_buf, wuv_buf, wo_buf, w1_buf, w2_buf,
               xs, t8, qa_ref, acc_ref, m_ref, l_ref, a_buf, e_buf, ctx_ref, mul_ref, o_buf,
               sem_w, sem_c, sem_o, sem_v, sem_small):
        cp = pltpu.make_async_copy

        def W(c, name):
            if TR:
                with jax.named_scope('@' + name):
                    c.wait()
            else:
                c.wait()

        def mark(name):
            if TR:
                with jax.named_scope('@' + name):
                    pl.delay(1)

        def loop(lo, hi, body):
            lax.fori_loop(lo, hi, lambda j, _: body(j), None)

        def piece(hbm, buf, a, r, n, sem, align=8):
            rows = pl.ds(r if isinstance(r, int) or align == 1 else pl.multiple_of(r, align), n)
            return cp(hbm.at[a, rows], buf.at[a, rows], sem)

        def issue_qk(lo, hi):
            def body(j):
                for r, n in PAT:
                    for a in range(4):
                        piece(wq_hbm, wq_buf, a, j * 8 + r // 8, n // 8, sem_w.at[0], 1).start(priority=0)
                        piece(wuk_hbm, wuk_buf, a, j * 8 + r // 8, n // 8, sem_w.at[1], 1).start(priority=1)
            loop(lo, hi, body)

        def issue_c(u, part=slice(None)):
            for r, n in PAT[part]:
                def body(t, r=r, n=n):
                    for i in range(8):
                        piece(ckv_hbm, c_buf, t * 4 + i // 2 + (i % 2) * 16, u * 64 + r, n, sem_c.at[u // 2]).start(priority=i % 2)
                loop(0, 4, body)

        def issue_v(lo, hi):
            def body(j):
                for t, (r, n) in enumerate(PAT):
                    for a in range(4):
                        piece(wuv_hbm, wuv_buf, a, j * 8 + r // 8, n // 8, sem_w.at[2], 1).start(priority=0)
                        if a % 2 == 1:
                            piece(w2_hbm, w2_buf, a // 2, j * 56 + W2P[t][0], W2P[t][1], sem_w.at[4]).start(priority=1)
                        elif t < 2:
                            piece(w1_hbm, w1_buf, a // 2, j * 16 + t * 8, 8, sem_w.at[3]).start(priority=1)
            loop(lo, hi, body)

        def issue_o(lo, hi):
            def body(j):
                for r, n in PAT:
                    for a in (0, 4, 2, 6, 1, 5, 3):
                        piece(wo_hbm, wo_buf, a, j * 64 + r, n, sem_o.at[(a // 4) * 4 + j // 2]).start(priority=a // 4)
            loop(lo, hi, body)

        cuts = (0,) + VC

        def issue_last():
            for i, (lo, hi) in enumerate(zip(cuts, cuts[1:])):
                for r in range(lo, hi, LP):
                    piece(wo_hbm, wo_buf, 7, r, min(LP, hi - r), sem_v.at[i]).start(priority=1)

        def wait_last(i):
            v = wo_buf.at[7, pl.ds(cuts[i], cuts[i + 1] - cuts[i])]
            W(cp(v, v, sem_v.at[i]), f'v{i}')

        x_cp = cp(x_hbm, x_buf, sem_small.at[0])
        b1_cp = cp(b1_hbm, b1_buf, sem_small.at[1])
        b2_cp = cp(b2_hbm, b2_buf, sem_small.at[2])

        issue_qk(0, 2)
        for c in (x_cp, b1_cp, b2_cp):
            c.start()
        issue_qk(2, 8)

        x_cp.wait()
        x = x_buf[...].astype(F32)
        xc = x - jnp.mean(x, axis=-1, keepdims=True)
        var = jnp.mean(xc * xc, axis=-1, keepdims=True)
        xn = (xc * lax.rsqrt(var + 1e-5)).astype(BF16)
        xf = xn.astype(F32)
        for b in range(B):
            for j in range(M // 128):
                xs[b, j * 128:(j + 1) * 128, :] = jnp.broadcast_to(xf[b:b + 1, j * 128:(j + 1) * 128], (128, 128)).T
        e_buf[...] = (lax.broadcasted_iota(jnp.int32, (128, 128 * H), 1) // H
                      == lax.broadcasted_iota(jnp.int32, (128, 128 * H), 0)).astype(F32).astype(BF16)
        mark('ln')
        issue_qk(8, 16)
        head, rest = slice(0, 1), slice(1, None)
        issue_c(0, head)
        issue_c(0, rest)

        W(cp(wq_buf, wq_buf, sem_w.at[0]), 'wq')
        issue_c(1, head)
        mark('q0')

        def q_body(i, carry):
            q0, q1 = carry
            for u in range(8):
                m = i * 8 + u
                w = wq_buf[i // 16, (i % 16) * 8 + u].astype(F32)
                q0 = q0 + xs[0, pl.ds(m, 1), :] * w
                q1 = q1 + xs[1, pl.ds(m, 1), :] * w
            return q0, q1

        q01 = lax.fori_loop(0, 32, q_body, (jnp.zeros((H, D), F32), jnp.zeros((H, D), F32)))
        issue_c(1, rest)
        q01 = lax.fori_loop(32, 64, q_body, q01)
        q = jnp.concatenate([q01[0], q01[1], jnp.zeros((128 - B * H, D), F32)], axis=0).astype(BF16)

        W(cp(wuk_buf, wuk_buf, sem_w.at[1]), 'wuk')
        group = (lax.broadcasted_iota(jnp.int32, (16, 8, 128), 2) % H) // 8

        def qa_body(i):
            pl.when(i % 2 == 0)(lambda: issue_c(2 + i // 2, head))
            pl.when(i % 2 == 1)(lambda: issue_c(2 + i // 2, rest))
            mark('qa')
            for u in range(8):
                w = wuk_buf[i, pl.ds(u * 16, 16)].reshape(16 * H, D)
                r = lax.dot_general(w, q, NT, preferred_element_type=F32).reshape(16, 4, 8, 128)
                v = jnp.where(group == 0, r[:, 0],
                              jnp.where(group == 1, r[:, 1], jnp.where(group == 2, r[:, 2], r[:, 3])))
                t8[pl.ds(pl.multiple_of((i * 8 + u) * 128, 128), 128), :] = v.reshape(128, 128)

        loop(0, 4, qa_body)
        issue_c(4, head)
        sub = lax.broadcasted_iota(jnp.int32, (128, 128), 1) % 8
        for j in range(DC // 128):
            t = t8[pl.ds(j * 1024, 128, stride=8), :]
            for s in range(1, 8):
                t = jnp.where(sub == s, t8[pl.ds(j * 1024 + s, 128, stride=8), :], t)
            qa_ref[:, j * 128:(j + 1) * 128] = (t.T[:B * H] * (D ** -0.5 * LOG2E)).astype(BF16)

        m_ref[...] = jnp.full((B * H, 128), -jnp.inf, F32)
        l_ref[...] = jnp.zeros((B * H, 128), F32)
        acc_ref[...] = jnp.zeros((B * H, DC), F32)

        def block(i):
            mark('blk')
            whole = i >= CU
            u = jnp.where(whole, i + 5 - CU // 2, 4 + (i + 1) // 2)
            pl.when(jnp.logical_and(jnp.logical_or(whole, i % 2 == 0), u <= NC))(lambda: issue_c(u - whole.astype(jnp.int32), rest))
            pl.when(jnp.logical_and(jnp.logical_or(whole, i % 2 == 1), u < NC))(lambda: issue_c(u, head))
            pl.when(u >= NC)(lambda: issue_v(jnp.maximum((u - NC) * 4 - 2, 0), (u - NC) * 4 + 2))
            g, b = i // 2, i % 2
            rows = pl.ds(pl.multiple_of(g * 128, 128), 128)
            pl.when(b == 0)(lambda: W(cp(c_buf.at[:, rows], c_buf.at[:, rows], sem_c.at[g]), 'c'))
            hrows = pl.ds(pl.multiple_of(b * H, H), H)
            c = c_buf[pl.ds(b * 16, 16), rows].reshape(BK, DC)
            sc = lax.dot_general(qa_ref[hrows, :], c, NT, preferred_element_type=F32)
            m_prev = m_ref[hrows, :]
            m_new = jnp.maximum(m_prev, jnp.max(sc, axis=1, keepdims=True))
            p = jnp.exp2(sc - m_new[:, :1])
            alpha = jnp.exp2(m_prev - m_new)
            l_ref[hrows, :] = alpha * l_ref[hrows, :] + jnp.sum(p, axis=1, keepdims=True)
            m_ref[hrows, :] = m_new
            pv = jnp.dot(p.astype(BF16), c, preferred_element_type=F32)
            acc_ref[hrows, :] = acc_ref[hrows, :] * alpha[:, :1] + pv

        loop(0, NC, block)
        mark('attn')
        if CU == 4: issue_v(10, 12)
        else: issue_v(14, 16)

        pc = (acc_ref[...] / l_ref[...][:, :1]).astype(BF16)
        diag = (lax.broadcasted_iota(jnp.int32, (B * H, 128 * H), 1) % H
                == lax.broadcasted_iota(jnp.int32, (B * H, 128 * H), 0) % H)
        for j in range(DC // 128):
            if j == 2:
                if CU == 4: issue_v(12, 14)
                else: issue_o(0, 2)
            rep = jnp.dot(pc[:, j * 128:(j + 1) * 128], e_buf[...], preferred_element_type=F32)
            a_buf[j] = jnp.where(diag, rep, 0.0).astype(BF16)
        mark('abuf')
        if CU == 4: issue_v(14, 16)
        issue_o(0 if CU == 4 else 2, 4)
        W(cp(wuv_buf, wuv_buf, sem_w.at[2]), 'wuv')
        ctx = jnp.zeros((B * H, D), F32)
        for j in range(DC // 128):
            if j == 2: issue_o(4, 5)
            ctx = ctx + jnp.dot(a_buf[j], wuv_buf[j].reshape(128 * H, D), preferred_element_type=F32)
        ctx_ref[:B * H] = ctx
        mark('ctx')
        issue_o(5, 7)
        cb = ctx.astype(BF16).astype(F32)
        for b in range(B):
            for k in range(V0 // D, 4):
                r = b * H + 28 + k
                mul_ref[b, k * D - V0:(k + 1) * D - V0] = jnp.broadcast_to(cb[r:r + 1], (128, 128)).T

        def rows8(v):
            return jnp.concatenate([v[:, j * 128:(j + 1) * 128] for j in range(4)], axis=0)

        issue_o(7, 8)
        W(cp(w1_buf, w1_buf, sem_w.at[3]), 'w1')
        cp(w2_buf, w2_buf, sem_w.at[4]).wait()
        b1_cp.wait()
        b2_cp.wait()
        hid = jnp.dot(xn, w1_buf[...].reshape(M, F), preferred_element_type=F32) + b1_buf[...].astype(F32).reshape(1, F)
        hid = jax.nn.gelu(hid, approximate=True).astype(BF16)
        z = jnp.dot(hid, w2_buf[...].reshape(F, M), preferred_element_type=F32) + b2_buf[...].astype(F32).reshape(1, M)
        z8 = rows8(z)
        g8 = z8 * jax.nn.sigmoid(z8)
        x8 = rows8(x)

        issue_last()

        def project(runs, h, n=1):
            lhs = jnp.concatenate([ctx_ref[pl.ds(4 * a + k, B, stride=H), :] for a in runs for k in range(h, h + n)], axis=1)
            rhs = wo_buf[runs[0]:runs[-1] + 1, h * D:(h + n) * D].reshape(len(runs) * n * D, M)
            return jnp.dot(lhs.astype(BF16), rhs, preferred_element_type=F32)

        s = None
        for p, h in ((0, 0), (0, 1), (1, 0), (0, 2), (0, 3), (1, 1), (1, 2), (1, 3)):
            runs = range(4, 7) if p else range(4)
            v = wo_buf.at[pl.ds(runs[0], len(runs)), pl.ds(h * D, D)]
            W(cp(v, v, sem_o.at[p * 4 + h]), f'o{p}{h}')
            t = project(runs, h)
            s = t if s is None else s + t
        wait_last(0)
        s = s + project(range(7, 8), 0, V0 // D)
        base8 = x8 + rows8(s) * g8
        acc = [[None] * 4 for _ in range(B)]
        for i in range(1, len(VC)):
            wait_last(i)
            for r in range(cuts[i], cuts[i + 1], 8):
                w = wo_buf[7, r:r + 8].astype(F32)
                for b in range(B):
                    mul = mul_ref[b, r - V0:r - V0 + 8, :]
                    for j in range(4):
                        pr = w[:, j * 128:(j + 1) * 128] * mul
                        acc[b][j] = pr if acc[b][j] is None else acc[b][j] + pr
        sl = lax.broadcasted_iota(jnp.int32, (8, 128), 0)

        def merge(a, c, k):
            m = (sl & k) != 0
            if k == 4:
                return jnp.where(m, c, a) + pltpu.roll(jnp.where(m, a, c), 4, 0)
            return jnp.where(m, c, a) + jnp.where(m, pltpu.roll(c, k, 0), pltpu.roll(a, 8 - k, 0))

        r4 = [[merge(acc[b][j], acc[b][j + 2], 4) for j in range(2)] for b in range(B)]
        r2 = [merge(r4[b][0], r4[b][1], 2) for b in range(B)]
        o_buf[...] = (base8 + g8 * merge(r2[0], r2[1], 1)).astype(BF16)
        done = cp(o_buf, o_hbm, sem_small.at[0])
        done.start()
        done.wait()

    def fn(A_x, A_c_kv, A_w_q, A_w_uk, A_w_uv, A_w_o, B_x, B_w1, B_b1, B_w2, B_b2):
        del B_x
        w4 = (4, 128, H, D)
        out = pl.pallas_call(
            kernel,
            out_shape=jax.ShapeDtypeStruct((8, 128), BF16),
            in_specs=[pl.BlockSpec(memory_space=pltpu.HBM)] * 10,
            out_specs=pl.BlockSpec(memory_space=pltpu.HBM),
            scratch_shapes=[
                pltpu.VMEM((B, M), BF16), pltpu.VMEM((F,), BF16), pltpu.VMEM((M,), BF16),
                pltpu.VMEM((32, 1024, DC), BF16),
                pltpu.VMEM(w4, BF16), pltpu.VMEM(w4, BF16), pltpu.VMEM(w4, BF16),
                pltpu.VMEM((8, 4 * D, M), BF16),
                pltpu.VMEM((2, M // 2, F), BF16), pltpu.VMEM((2, F // 2, M), BF16),
                pltpu.VMEM((B, M, 128), F32),
                pltpu.VMEM((DC * 8 + 8, 128), F32),
                pltpu.VMEM((B * H, DC), BF16), pltpu.VMEM((B * H, DC), F32),
                pltpu.VMEM((B * H, 128), F32), pltpu.VMEM((B * H, 128), F32),
                pltpu.VMEM((4, B * H, 128 * H), BF16), pltpu.VMEM((128, 128 * H), BF16),
                pltpu.VMEM((3 * H, D), F32), pltpu.VMEM((B, 512 - V0, 128), F32), pltpu.VMEM((8, 128), BF16),
                pltpu.SemaphoreType.DMA((5,)), pltpu.SemaphoreType.DMA((8,)), pltpu.SemaphoreType.DMA((8,)),
                pltpu.SemaphoreType.DMA((len(VC),)), pltpu.SemaphoreType.DMA((3,)),
            ],
            compiler_params=pltpu.CompilerParams(vmem_limit_bytes=100 * 1024 * 1024, flags=flags,
                                                 disable_semaphore_checks=True, disable_bounds_checks=True),
        )(A_x.reshape(B, M), A_c_kv.reshape(32, 1024, DC), A_w_q.reshape(w4), A_w_uk.reshape(w4),
          A_w_uv.reshape(w4), A_w_o.reshape(8, 4 * D, M), B_w1.reshape(2, M // 2, F), B_b1, B_w2.reshape(2, F // 2, M), B_b2)
        return out.reshape(4, B, 128).transpose(1, 0, 2).reshape(B, 1, M)
    return fn


_impl = make(LP=32)


@jax.jit
def pallas_recurrent_scan__compressed_kv_cla__dense_activation_gelu__decode_kernel(
    A_x, A_c_kv, A_w_q, A_w_uk, A_w_uv, A_w_o, B_x, B_w1, B_b1, B_w2, B_b2,
):
    return _impl(A_x, A_c_kv, A_w_q, A_w_uk, A_w_uv, A_w_o, B_x, B_w1, B_b1, B_w2, B_b2)
```

```python
import jax
import jax.numpy as jnp
from jax import lax
import jax.experimental.pallas as pl
import jax.experimental.pallas.tpu as pltpu

F32 = jnp.float32
BF16 = jnp.bfloat16

B, H, SK, D, M, DC, F = 2, 32, 16384, 128, 512, 512, 1792
LOG2E = 1.4426950408889634
NT = (((1,), (1,)), ((), ()))

PIECES = ((0, 32), (32, 16), (48, 16))
W2_PIECES = ((0, 24), (24, 16), (40, 16))
QK_VIEW = (8, 64, H, D)
UV_VIEW = (4, 128, H, D)
C_RUNS = 16
C_VIEW = (B * C_RUNS, SK // C_RUNS, DC)
C_ROUNDS = SK // C_RUNS // 64
O_VIEW = (8, 4 * D, M)
BK = 128 * C_RUNS
LAST_CUTS = (0, D, 320, 384, 448, 496, 512)


def _loop(lo, hi, body):
    lax.fori_loop(lo, hi, lambda i, _: body(i), None)


def _rows8(v):
    return jnp.concatenate([v[:, j * 128:(j + 1) * 128] for j in range(M // 128)], axis=0)


def _kernel(x_hbm, ckv_hbm, wq_hbm, wuk_hbm, wuv_hbm, wo_hbm, w1_hbm, b1_hbm, w2_hbm, b2_hbm,
            o_hbm,
            x_buf, b1_buf, b2_buf, c_buf, wq_buf, wuk_buf, wuv_buf, wo_buf, w1_buf, w2_buf,
            xs, t8, qa_ref, acc_ref, m_ref, l_ref, a_buf, e_buf, ctx_ref, mul_ref, o_buf,
            sem_w, sem_c, sem_o, sem_last, sem_small):
    def fetch(hbm, buf, run, row, n, sem, queue):
        rows = pl.ds(row, n)
        pltpu.make_async_copy(hbm.at[run, rows], buf.at[run, rows], sem).start(priority=queue)

    def wait_filled(buf, sem):
        pltpu.make_async_copy(buf, buf, sem).wait()

    def issue_qk(lo, hi):
        def body(j):
            for r, n in PIECES:
                for a in range(QK_VIEW[0]):
                    fetch(wq_hbm, wq_buf, a, j * 8 + r // 8, n // 8, sem_w.at[0], 0)
                    fetch(wuk_hbm, wuk_buf, a, j * 8 + r // 8, n // 8, sem_w.at[1], 1)
        _loop(lo, hi, body)

    head, rest = PIECES[:1], PIECES[1:]

    def issue_c(j, pieces):
        for r, n in pieces:
            row = j * 64 + r if isinstance(j, int) else pl.multiple_of(j * 64 + r, 16)

            def body(t):
                for i in range(8):
                    b = i % 2
                    fetch(ckv_hbm, c_buf, b * C_RUNS + t * 4 + i // 2, row, n, sem_c.at[j // 2], b)
            _loop(0, C_RUNS // 4, body)

    def issue_v(lo, hi):
        def body(j):
            for t, (r, n) in enumerate(PIECES):
                for a in range(UV_VIEW[0]):
                    fetch(wuv_hbm, wuv_buf, a, j * 8 + r // 8, n // 8, sem_w.at[2], 0)
                    if a % 2 == 1:
                        row = pl.multiple_of(j * 56 + W2_PIECES[t][0], 8)
                        fetch(w2_hbm, w2_buf, a // 2, row, W2_PIECES[t][1], sem_w.at[4], 1)
                    elif t < 2:
                        fetch(w1_hbm, w1_buf, a // 2, pl.multiple_of(j * 16 + t * 8, 8), 8, sem_w.at[3], 1)
        _loop(lo, hi, body)

    def issue_o(lo, hi):
        def body(j):
            for r, n in PIECES:
                for a in (0, 4, 2, 6, 1, 5, 3):
                    fetch(wo_hbm, wo_buf, a, pl.multiple_of(j * 64 + r, 16), n,
                          sem_o.at[(a // 4) * 4 + j // 2], a // 4)
        _loop(lo, hi, body)

    def issue_last():
        for i, (lo, hi) in enumerate(zip(LAST_CUTS, LAST_CUTS[1:])):
            for r in range(lo, hi, 32):
                fetch(wo_hbm, wo_buf, 7, r, min(32, hi - r), sem_last.at[i], 1)

    x_copy = pltpu.make_async_copy(x_hbm, x_buf, sem_small.at[0])
    b1_copy = pltpu.make_async_copy(b1_hbm, b1_buf, sem_small.at[1])
    b2_copy = pltpu.make_async_copy(b2_hbm, b2_buf, sem_small.at[2])

    issue_qk(0, 1)
    for c in (x_copy, b1_copy, b2_copy):
        c.start()
    issue_qk(1, 4)

    x_copy.wait()
    x = x_buf[...].astype(F32)
    xc = x - jnp.mean(x, axis=-1, keepdims=True)
    var = jnp.mean(xc * xc, axis=-1, keepdims=True)
    xn = (xc * lax.rsqrt(var + 1e-5)).astype(BF16)
    xf = xn.astype(F32)
    for b in range(B):
        for j in range(M // 128):
            cols = slice(j * 128, (j + 1) * 128)
            xs[b, cols, :] = jnp.broadcast_to(xf[b:b + 1, cols], (128, 128)).T
    e_buf[...] = (lax.broadcasted_iota(jnp.int32, (128, 128 * H), 1) // H
                  == lax.broadcasted_iota(jnp.int32, (128, 128 * H), 0)).astype(F32).astype(BF16)
    issue_qk(4, 8)
    issue_c(0, PIECES)

    wait_filled(wq_buf, sem_w.at[0])

    def q_body(i, carry):
        q0, q1 = carry
        for u in range(8):
            m = pl.ds(i * 8 + u, 1)
            w = wq_buf[i // 8, (i % 8) * 8 + u].astype(F32)
            q0 = q0 + xs[0, m, :] * w
            q1 = q1 + xs[1, m, :] * w
        return q0, q1

    issue_c(1, head)
    q01 = lax.fori_loop(0, 32, q_body, (jnp.zeros((H, D), F32), jnp.zeros((H, D), F32)))
    issue_c(1, rest)
    q0, q1 = lax.fori_loop(32, 64, q_body, q01)
    q = jnp.concatenate([q0, q1, jnp.zeros((128 - B * H, D), F32)], axis=0).astype(BF16)

    wait_filled(wuk_buf, sem_w.at[1])
    group = (lax.broadcasted_iota(jnp.int32, (16, 8, 128), 2) % H) // 8

    def qa_body(i):
        pl.when(i % 2 == 0)(lambda: issue_c(2 + i // 2, head))
        pl.when(i % 2 == 1)(lambda: issue_c(2 + i // 2, rest))
        for u in range(8):
            w = wuk_buf[2 * i + u // 4, pl.ds((u % 4) * 16, 16)].reshape(16 * H, D)
            r = lax.dot_general(w, q, NT, preferred_element_type=F32).reshape(16, 4, 8, 128)
            v = jnp.where(group == 0, r[:, 0],
                          jnp.where(group == 1, r[:, 1], jnp.where(group == 2, r[:, 2], r[:, 3])))
            t8[pl.ds(pl.multiple_of((i * 8 + u) * 128, 128), 128), :] = v.reshape(128, 128)

    _loop(0, 4, qa_body)
    issue_c(4, head)
    sub = lax.broadcasted_iota(jnp.int32, (128, 128), 1) % 8
    for j in range(DC // 128):
        t = t8[pl.ds(j * 1024, 128, stride=8), :]
        for s in range(1, 8):
            t = jnp.where(sub == s, t8[pl.ds(j * 1024 + s, 128, stride=8), :], t)
        qa_ref[:, j * 128:(j + 1) * 128] = (t.T[:B * H] * (D ** -0.5 * LOG2E)).astype(BF16)

    m_ref[...] = jnp.full((B * H, 128), -jnp.inf, F32)
    l_ref[...] = jnp.zeros((B * H, 128), F32)
    acc_ref[...] = jnp.zeros((B * H, DC), F32)

    def block(i):
        j = i + 4
        pl.when(jnp.logical_and(i != 1, j <= C_ROUNDS))(lambda: issue_c(jnp.maximum(j - 1, 4), rest))
        pl.when(jnp.logical_and(i != 0, j < C_ROUNDS))(lambda: issue_c(j, head))
        pl.when(j >= C_ROUNDS)(
            lambda: issue_v(jnp.maximum((j - C_ROUNDS) * 4 - 2, 0), (j - C_ROUNDS) * 4 + 2))

        g, b = i // B, i % B
        rows = pl.ds(pl.multiple_of(g * 128, 128), 128)
        pl.when(b == 0)(lambda: wait_filled(c_buf.at[:, rows], sem_c.at[g]))
        hrows = pl.ds(pl.multiple_of(b * H, H), H)
        c = c_buf[pl.ds(b * C_RUNS, C_RUNS), rows].reshape(BK, DC)
        sc = lax.dot_general(qa_ref[hrows, :], c, NT, preferred_element_type=F32)
        m_prev = m_ref[hrows, :]
        m_new = jnp.maximum(m_prev, jnp.max(sc, axis=1, keepdims=True))
        p = jnp.exp2(sc - m_new[:, :1])
        alpha = jnp.exp2(m_prev - m_new)
        l_ref[hrows, :] = alpha * l_ref[hrows, :] + jnp.sum(p, axis=1, keepdims=True)
        m_ref[hrows, :] = m_new
        pv = jnp.dot(p.astype(BF16), c, preferred_element_type=F32)
        acc_ref[hrows, :] = acc_ref[hrows, :] * alpha[:, :1] + pv

    _loop(0, B * SK // BK, block)
    issue_v(14, 16)

    pc = (acc_ref[...] / l_ref[...][:, :1]).astype(BF16)
    diag = (lax.broadcasted_iota(jnp.int32, (B * H, 128 * H), 1) % H
            == lax.broadcasted_iota(jnp.int32, (B * H, 128 * H), 0) % H)
    for j in range(DC // 128):
        if j == 2:
            issue_o(0, 2)
        rep = jnp.dot(pc[:, j * 128:(j + 1) * 128], e_buf[...], preferred_element_type=F32)
        a_buf[j] = jnp.where(diag, rep, 0.0).astype(BF16)
    issue_o(2, 4)
    wait_filled(wuv_buf, sem_w.at[2])
    ctx = jnp.zeros((B * H, D), F32)
    for j in range(DC // 128):
        if j == 2:
            issue_o(4, 5)
        ctx = ctx + jnp.dot(a_buf[j], wuv_buf[j].reshape(128 * H, D), preferred_element_type=F32)
    ctx_ref[:B * H] = ctx
    issue_o(5, 7)
    cb = ctx.astype(BF16).astype(F32)
    for b in range(B):
        for k in range(1, 4):
            r = b * H + H - 4 + k
            mul_ref[b, (k - 1) * D:k * D] = jnp.broadcast_to(cb[r:r + 1], (128, 128)).T
    issue_o(7, 8)

    wait_filled(w1_buf, sem_w.at[3])
    wait_filled(w2_buf, sem_w.at[4])
    b1_copy.wait()
    b2_copy.wait()
    hid = jnp.dot(xn, w1_buf[...].reshape(M, F), preferred_element_type=F32)
    hid = jax.nn.gelu(hid + b1_buf[...].astype(F32).reshape(1, F), approximate=True).astype(BF16)
    z = jnp.dot(hid, w2_buf[...].reshape(F, M), preferred_element_type=F32)
    z8 = _rows8(z + b2_buf[...].astype(F32).reshape(1, M))
    g8 = z8 * jax.nn.sigmoid(z8)
    x8 = _rows8(x)
    issue_last()

    def project(parts):
        lhs = jnp.concatenate([ctx_ref[pl.ds(4 * a + k, B, stride=H), :]
                               for a0, n, k in parts for a in range(a0, a0 + n)], axis=1)
        rhs = jnp.concatenate([wo_buf[a0:a0 + n, k * D:(k + 1) * D].reshape(n * D, M)
                               for a0, n, k in parts], axis=0)
        return jnp.dot(lhs.astype(BF16), rhs, preferred_element_type=F32)

    def wait_last(i):
        wait_filled(wo_buf.at[7, pl.ds(LAST_CUTS[i], LAST_CUTS[i + 1] - LAST_CUTS[i])], sem_last.at[i])

    s = jnp.zeros((B, M), F32)
    for step in (((0, 4, 0), (0, 4, 1), (4, 3, 0)), ((0, 4, 2), (0, 4, 3), (4, 3, 1)), ((4, 3, 2),), ((4, 3, 3),)):
        for a0, n, k in step:
            wait_filled(wo_buf.at[pl.ds(a0, n), pl.ds(k * D, D)], sem_o.at[a0 + k])
        s = s + project(step)
    wait_last(0)
    base8 = x8 + _rows8(s + project(((7, 1, 0),))) * g8

    part = [[None] * (M // 128) for _ in range(B)]
    for i in range(1, len(LAST_CUTS) - 1):
        wait_last(i)
        for r in range(LAST_CUTS[i], LAST_CUTS[i + 1], 8):
            w = wo_buf[7, r:r + 8].astype(F32)
            for b in range(B):
                mul = mul_ref[b, r - D:r - D + 8, :]
                for j in range(M // 128):
                    t = w[:, j * 128:(j + 1) * 128] * mul
                    part[b][j] = t if part[b][j] is None else part[b][j] + t

    sl = lax.broadcasted_iota(jnp.int32, (8, 128), 0)

    def merge(lo, hi, k):
        m = (sl & k) != 0
        if k == 4:
            return jnp.where(m, hi, lo) + pltpu.roll(jnp.where(m, lo, hi), 4, 0)
        return jnp.where(m, hi, lo) + jnp.where(m, pltpu.roll(hi, k, 0), pltpu.roll(lo, 8 - k, 0))

    r4 = [[merge(part[b][j], part[b][j + 2], 4) for j in range(2)] for b in range(B)]
    r2 = [merge(r4[b][0], r4[b][1], 2) for b in range(B)]
    o_buf[...] = (base8 + g8 * merge(r2[0], r2[1], 1)).astype(BF16)
    o_copy = pltpu.make_async_copy(o_buf, o_hbm, sem_small.at[0])
    o_copy.start()
    o_copy.wait()


@jax.jit
def pallas_recurrent_scan__compressed_kv_cla__dense_activation_gelu__decode_kernel(
    A_x: jax.Array,
    A_c_kv: jax.Array,
    A_w_q: jax.Array,
    A_w_uk: jax.Array,
    A_w_uv: jax.Array,
    A_w_o: jax.Array,
    B_x: jax.Array,
    B_w1: jax.Array,
    B_b1: jax.Array,
    B_w2: jax.Array,
    B_b2: jax.Array,
):
    del B_x
    hbm = pl.BlockSpec(memory_space=pltpu.HBM)
    dma_sems = pltpu.SemaphoreType.DMA
    w1_view, w2_view = (2, M // 2, F), (2, F // 2, M)
    out = pl.pallas_call(
        _kernel,
        out_shape=jax.ShapeDtypeStruct((8, 128), BF16),
        in_specs=[hbm] * 10,
        out_specs=hbm,
        scratch_shapes=[
            pltpu.VMEM((B, M), BF16), pltpu.VMEM((F,), BF16), pltpu.VMEM((M,), BF16),
            pltpu.VMEM(C_VIEW, BF16), pltpu.VMEM(QK_VIEW, BF16), pltpu.VMEM(QK_VIEW, BF16),
            pltpu.VMEM(UV_VIEW, BF16), pltpu.VMEM(O_VIEW, BF16),
            pltpu.VMEM(w1_view, BF16), pltpu.VMEM(w2_view, BF16),
            pltpu.VMEM((B, M, 128), F32),
            pltpu.VMEM((DC * 8 + 8, 128), F32),
            pltpu.VMEM((B * H, DC), BF16), pltpu.VMEM((B * H, DC), F32),
            pltpu.VMEM((B * H, 128), F32), pltpu.VMEM((B * H, 128), F32),
            pltpu.VMEM((DC // 128, B * H, 128 * H), BF16), pltpu.VMEM((128, 128 * H), BF16),
            pltpu.VMEM((3 * H, D), F32), pltpu.VMEM((B, 3 * D, 128), F32), pltpu.VMEM((8, 128), BF16),
            dma_sems((5,)), dma_sems((C_ROUNDS // 2,)), dma_sems((8,)), dma_sems((len(LAST_CUTS) - 1,)),
            dma_sems((3,)),
        ],
        compiler_params=pltpu.CompilerParams(
            vmem_limit_bytes=100 * 1024 * 1024, disable_semaphore_checks=True, disable_bounds_checks=True),
    )(A_x.reshape(B, M), A_c_kv.reshape(C_VIEW), A_w_q.reshape(QK_VIEW), A_w_uk.reshape(QK_VIEW),
      A_w_uv.reshape(UV_VIEW), A_w_o.reshape(O_VIEW), B_w1.reshape(w1_view), B_b1, B_w2.reshape(w2_view), B_b2)
    return out.reshape(M // 128, B, 128).transpose(1, 0, 2).reshape(B, 1, M)
```

```python
import jax
import jax.numpy as jnp
from jax import lax
import jax.experimental.pallas as pl
import jax.experimental.pallas.tpu as pltpu

F32 = jnp.float32
BF16 = jnp.bfloat16

B, H, SK, D, M, DC, F = 2, 32, 16384, 128, 512, 512, 1792
LOG2E = 1.4426950408889634
NT = (((1,), (1,)), ((), ()))

PIECES = ((0, 32), (32, 16), (48, 16))
W2_PIECES = ((0, 24), (24, 16), (40, 16))
W_VIEW = (4, 128, H, D)
C_RUNS = 16
C_VIEW = (B * C_RUNS, SK // C_RUNS, DC)
C_ROUNDS = SK // C_RUNS // 64
O_VIEW = (8, 4 * D, M)
BK = 128 * C_RUNS
LAST_CUTS = (0, D, 320, 384, 448, 496, 512)


def _loop(lo, hi, body):
    lax.fori_loop(lo, hi, lambda i, _: body(i), None)


def _rows8(v):
    return jnp.concatenate([v[:, j * 128:(j + 1) * 128] for j in range(M // 128)], axis=0)


def _kernel(x_hbm, ckv_hbm, wq_hbm, wuk_hbm, wuv_hbm, wo_hbm, w1_hbm, b1_hbm, w2_hbm, b2_hbm,
            o_hbm,
            x_buf, b1_buf, b2_buf, c_buf, wq_buf, wuk_buf, wuv_buf, wo_buf, w1_buf, w2_buf,
            xs, t8, qa_ref, acc_ref, m_ref, l_ref, a_buf, e_buf, ctx_ref, mul_ref, o_buf,
            sem_w, sem_c, sem_o, sem_last, sem_small):
    def fetch(hbm, buf, run, row, n, sem, queue):
        rows = pl.ds(row, n)
        pltpu.make_async_copy(hbm.at[run, rows], buf.at[run, rows], sem).start(priority=queue)

    def wait_filled(buf, sem):
        pltpu.make_async_copy(buf, buf, sem).wait()

    def issue_qk(lo, hi):
        def body(j):
            for r, n in PIECES:
                for a in range(W_VIEW[0]):
                    fetch(wq_hbm, wq_buf, a, j * 8 + r // 8, n // 8, sem_w.at[0], 0)
                    fetch(wuk_hbm, wuk_buf, a, j * 8 + r // 8, n // 8, sem_w.at[1], 1)
        _loop(lo, hi, body)

    head, rest = PIECES[:1], PIECES[1:]

    def issue_c(j, pieces):
        for r, n in pieces:
            row = j * 64 + r if isinstance(j, int) else pl.multiple_of(j * 64 + r, 16)

            def body(t):
                for i in range(8):
                    b = i % 2
                    fetch(ckv_hbm, c_buf, b * C_RUNS + t * 4 + i // 2, row, n, sem_c.at[j // 2], b)
            _loop(0, C_RUNS // 4, body)

    def issue_v(lo, hi):
        def body(j):
            for t, (r, n) in enumerate(PIECES):
                for a in range(W_VIEW[0]):
                    fetch(wuv_hbm, wuv_buf, a, j * 8 + r // 8, n // 8, sem_w.at[2], 0)
                    if a % 2 == 1:
                        row = pl.multiple_of(j * 56 + W2_PIECES[t][0], 8)
                        fetch(w2_hbm, w2_buf, a // 2, row, W2_PIECES[t][1], sem_w.at[4], 1)
                    elif t < 2:
                        fetch(w1_hbm, w1_buf, a // 2, pl.multiple_of(j * 16 + t * 8, 8), 8, sem_w.at[3], 1)
        _loop(lo, hi, body)

    def issue_o(lo, hi):
        def body(j):
            for r, n in PIECES:
                for a in (0, 4, 2, 6, 1, 5, 3):
                    fetch(wo_hbm, wo_buf, a, pl.multiple_of(j * 64 + r, 16), n,
                          sem_o.at[(a // 4) * 4 + j // 2], a // 4)
        _loop(lo, hi, body)

    def issue_last():
        for i, (lo, hi) in enumerate(zip(LAST_CUTS, LAST_CUTS[1:])):
            for r in range(lo, hi, 32):
                fetch(wo_hbm, wo_buf, 7, r, min(32, hi - r), sem_last.at[i], 1)

    x_copy = pltpu.make_async_copy(x_hbm, x_buf, sem_small.at[0])
    b1_copy = pltpu.make_async_copy(b1_hbm, b1_buf, sem_small.at[1])
    b2_copy = pltpu.make_async_copy(b2_hbm, b2_buf, sem_small.at[2])

    issue_qk(0, 2)
    for c in (x_copy, b1_copy, b2_copy):
        c.start()
    issue_qk(2, 8)

    x_copy.wait()
    x = x_buf[...].astype(F32)
    xc = x - jnp.mean(x, axis=-1, keepdims=True)
    var = jnp.mean(xc * xc, axis=-1, keepdims=True)
    xn = (xc * lax.rsqrt(var + 1e-5)).astype(BF16)
    xf = xn.astype(F32)
    for b in range(B):
        for j in range(M // 128):
            cols = slice(j * 128, (j + 1) * 128)
            xs[b, cols, :] = jnp.broadcast_to(xf[b:b + 1, cols], (128, 128)).T
    e_buf[...] = (lax.broadcasted_iota(jnp.int32, (128, 128 * H), 1) // H
                  == lax.broadcasted_iota(jnp.int32, (128, 128 * H), 0)).astype(F32).astype(BF16)
    issue_qk(8, 16)
    issue_c(0, PIECES)

    wait_filled(wq_buf, sem_w.at[0])

    def q_body(i, carry):
        q0, q1 = carry
        for u in range(8):
            m = pl.ds(i * 8 + u, 1)
            w = wq_buf[i // 16, (i % 16) * 8 + u].astype(F32)
            q0 = q0 + xs[0, m, :] * w
            q1 = q1 + xs[1, m, :] * w
        return q0, q1

    issue_c(1, head)
    q01 = lax.fori_loop(0, 32, q_body, (jnp.zeros((H, D), F32), jnp.zeros((H, D), F32)))
    issue_c(1, rest)
    q0, q1 = lax.fori_loop(32, 64, q_body, q01)
    q = jnp.concatenate([q0, q1, jnp.zeros((128 - B * H, D), F32)], axis=0).astype(BF16)

    wait_filled(wuk_buf, sem_w.at[1])
    group = (lax.broadcasted_iota(jnp.int32, (16, 8, 128), 2) % H) // 8

    def qa_body(i):
        pl.when(i % 2 == 0)(lambda: issue_c(2 + i // 2, head))
        pl.when(i % 2 == 1)(lambda: issue_c(2 + i // 2, rest))
        for u in range(8):
            w = wuk_buf[i, pl.ds(u * 16, 16)].reshape(16 * H, D)
            r = lax.dot_general(w, q, NT, preferred_element_type=F32).reshape(16, 4, 8, 128)
            v = jnp.where(group == 0, r[:, 0],
                          jnp.where(group == 1, r[:, 1], jnp.where(group == 2, r[:, 2], r[:, 3])))
            t8[pl.ds(pl.multiple_of((i * 8 + u) * 128, 128), 128), :] = v.reshape(128, 128)

    _loop(0, 4, qa_body)
    issue_c(4, head)
    sub = lax.broadcasted_iota(jnp.int32, (128, 128), 1) % 8
    for j in range(DC // 128):
        t = t8[pl.ds(j * 1024, 128, stride=8), :]
        for s in range(1, 8):
            t = jnp.where(sub == s, t8[pl.ds(j * 1024 + s, 128, stride=8), :], t)
        qa_ref[:, j * 128:(j + 1) * 128] = (t.T[:B * H] * (D ** -0.5 * LOG2E)).astype(BF16)

    m_ref[...] = jnp.full((B * H, 128), -jnp.inf, F32)
    l_ref[...] = jnp.zeros((B * H, 128), F32)
    acc_ref[...] = jnp.zeros((B * H, DC), F32)

    def block(i):
        j = i + 4
        pl.when(jnp.logical_and(i != 1, j <= C_ROUNDS))(lambda: issue_c(jnp.maximum(j - 1, 4), rest))
        pl.when(jnp.logical_and(i != 0, j < C_ROUNDS))(lambda: issue_c(j, head))
        pl.when(j >= C_ROUNDS)(
            lambda: issue_v(jnp.maximum((j - C_ROUNDS) * 4 - 2, 0), (j - C_ROUNDS) * 4 + 2))

        g, b = i // B, i % B
        rows = pl.ds(pl.multiple_of(g * 128, 128), 128)
        pl.when(b == 0)(lambda: wait_filled(c_buf.at[:, rows], sem_c.at[g]))
        hrows = pl.ds(pl.multiple_of(b * H, H), H)
        c = c_buf[pl.ds(b * C_RUNS, C_RUNS), rows].reshape(BK, DC)
        sc = lax.dot_general(qa_ref[hrows, :], c, NT, preferred_element_type=F32)
        m_prev = m_ref[hrows, :]
        m_new = jnp.maximum(m_prev, jnp.max(sc, axis=1, keepdims=True))
        p = jnp.exp2(sc - m_new[:, :1])
        alpha = jnp.exp2(m_prev - m_new)
        l_ref[hrows, :] = alpha * l_ref[hrows, :] + jnp.sum(p, axis=1, keepdims=True)
        m_ref[hrows, :] = m_new
        pv = jnp.dot(p.astype(BF16), c, preferred_element_type=F32)
        acc_ref[hrows, :] = acc_ref[hrows, :] * alpha[:, :1] + pv

    _loop(0, B * SK // BK, block)
    issue_v(14, 16)

    pc = (acc_ref[...] / l_ref[...][:, :1]).astype(BF16)
    diag = (lax.broadcasted_iota(jnp.int32, (B * H, 128 * H), 1) % H
            == lax.broadcasted_iota(jnp.int32, (B * H, 128 * H), 0) % H)
    for j in range(DC // 128):
        if j == 2:
            issue_o(0, 2)
        rep = jnp.dot(pc[:, j * 128:(j + 1) * 128], e_buf[...], preferred_element_type=F32)
        a_buf[j] = jnp.where(diag, rep, 0.0).astype(BF16)
    issue_o(2, 4)
    wait_filled(wuv_buf, sem_w.at[2])
    ctx = jnp.zeros((B * H, D), F32)
    for j in range(DC // 128):
        if j == 2:
            issue_o(4, 5)
        ctx = ctx + jnp.dot(a_buf[j], wuv_buf[j].reshape(128 * H, D), preferred_element_type=F32)
    ctx_ref[:B * H] = ctx
    issue_o(5, 7)
    cb = ctx.astype(BF16).astype(F32)
    for b in range(B):
        for k in range(1, 4):
            r = b * H + H - 4 + k
            mul_ref[b, (k - 1) * D:k * D] = jnp.broadcast_to(cb[r:r + 1], (128, 128)).T
    issue_o(7, 8)

    wait_filled(w1_buf, sem_w.at[3])
    wait_filled(w2_buf, sem_w.at[4])
    b1_copy.wait()
    b2_copy.wait()
    hid = jnp.dot(xn, w1_buf[...].reshape(M, F), preferred_element_type=F32)
    hid = jax.nn.gelu(hid + b1_buf[...].astype(F32).reshape(1, F), approximate=True).astype(BF16)
    z = jnp.dot(hid, w2_buf[...].reshape(F, M), preferred_element_type=F32)
    z8 = _rows8(z + b2_buf[...].astype(F32).reshape(1, M))
    g8 = z8 * jax.nn.sigmoid(z8)
    x8 = _rows8(x)
    issue_last()

    def project(parts):
        lhs = jnp.concatenate([ctx_ref[pl.ds(4 * a + k, B, stride=H), :]
                               for a0, n, k in parts for a in range(a0, a0 + n)], axis=1)
        rhs = jnp.concatenate([wo_buf[a0:a0 + n, k * D:(k + 1) * D].reshape(n * D, M)
                               for a0, n, k in parts], axis=0)
        return jnp.dot(lhs.astype(BF16), rhs, preferred_element_type=F32)

    def wait_last(i):
        wait_filled(wo_buf.at[7, pl.ds(LAST_CUTS[i], LAST_CUTS[i + 1] - LAST_CUTS[i])], sem_last.at[i])

    s = jnp.zeros((B, M), F32)
    for step in (((0, 4, 0), (0, 4, 1), (4, 3, 0)), ((0, 4, 2), (0, 4, 3), (4, 3, 1)), ((4, 3, 2),), ((4, 3, 3),)):
        for a0, n, k in step:
            wait_filled(wo_buf.at[pl.ds(a0, n), pl.ds(k * D, D)], sem_o.at[a0 + k])
        s = s + project(step)
    wait_last(0)
    base8 = x8 + _rows8(s + project(((7, 1, 0),))) * g8

    part = [[None] * (M // 128) for _ in range(B)]
    for i in range(1, len(LAST_CUTS) - 1):
        wait_last(i)
        for r in range(LAST_CUTS[i], LAST_CUTS[i + 1], 8):
            w = wo_buf[7, r:r + 8].astype(F32)
            for b in range(B):
                mul = mul_ref[b, r - D:r - D + 8, :]
                for j in range(M // 128):
                    t = w[:, j * 128:(j + 1) * 128] * mul
                    part[b][j] = t if part[b][j] is None else part[b][j] + t

    sl = lax.broadcasted_iota(jnp.int32, (8, 128), 0)

    def merge(lo, hi, k):
        m = (sl & k) != 0
        if k == 4:
            return jnp.where(m, hi, lo) + pltpu.roll(jnp.where(m, lo, hi), 4, 0)
        return jnp.where(m, hi, lo) + jnp.where(m, pltpu.roll(hi, k, 0), pltpu.roll(lo, 8 - k, 0))

    r4 = [[merge(part[b][j], part[b][j + 2], 4) for j in range(2)] for b in range(B)]
    r2 = [merge(r4[b][0], r4[b][1], 2) for b in range(B)]
    o_buf[...] = (base8 + g8 * merge(r2[0], r2[1], 1)).astype(BF16)
    o_copy = pltpu.make_async_copy(o_buf, o_hbm, sem_small.at[0])
    o_copy.start()
    o_copy.wait()


@jax.jit
def pallas_recurrent_scan__compressed_kv_cla__dense_activation_gelu__decode_kernel(
    A_x: jax.Array,
    A_c_kv: jax.Array,
    A_w_q: jax.Array,
    A_w_uk: jax.Array,
    A_w_uv: jax.Array,
    A_w_o: jax.Array,
    B_x: jax.Array,
    B_w1: jax.Array,
    B_b1: jax.Array,
    B_w2: jax.Array,
    B_b2: jax.Array,
):
    del B_x
    hbm = pl.BlockSpec(memory_space=pltpu.HBM)
    dma_sems = pltpu.SemaphoreType.DMA
    w1_view, w2_view = (2, M // 2, F), (2, F // 2, M)
    out = pl.pallas_call(
        _kernel,
        out_shape=jax.ShapeDtypeStruct((8, 128), BF16),
        in_specs=[hbm] * 10,
        out_specs=hbm,
        scratch_shapes=[
            pltpu.VMEM((B, M), BF16), pltpu.VMEM((F,), BF16), pltpu.VMEM((M,), BF16),
            pltpu.VMEM(C_VIEW, BF16), pltpu.VMEM(W_VIEW, BF16), pltpu.VMEM(W_VIEW, BF16),
            pltpu.VMEM(W_VIEW, BF16), pltpu.VMEM(O_VIEW, BF16),
            pltpu.VMEM(w1_view, BF16), pltpu.VMEM(w2_view, BF16),
            pltpu.VMEM((B, M, 128), F32),
            pltpu.VMEM((DC * 8 + 8, 128), F32),
            pltpu.VMEM((B * H, DC), BF16), pltpu.VMEM((B * H, DC), F32),
            pltpu.VMEM((B * H, 128), F32), pltpu.VMEM((B * H, 128), F32),
            pltpu.VMEM((DC // 128, B * H, 128 * H), BF16), pltpu.VMEM((128, 128 * H), BF16),
            pltpu.VMEM((3 * H, D), F32), pltpu.VMEM((B, 3 * D, 128), F32), pltpu.VMEM((8, 128), BF16),
            dma_sems((5,)), dma_sems((C_ROUNDS // 2,)), dma_sems((8,)), dma_sems((len(LAST_CUTS) - 1,)),
            dma_sems((3,)),
        ],
        compiler_params=pltpu.CompilerParams(
            vmem_limit_bytes=100 * 1024 * 1024, disable_semaphore_checks=True, disable_bounds_checks=True),
    )(A_x.reshape(B, M), A_c_kv.reshape(C_VIEW), A_w_q.reshape(W_VIEW), A_w_uk.reshape(W_VIEW),
      A_w_uv.reshape(W_VIEW), A_w_o.reshape(O_VIEW), B_w1.reshape(w1_view), B_b1, B_w2.reshape(w2_view), B_b2)
    return out.reshape(M // 128, B, 128).transpose(1, 0, 2).reshape(B, 1, M)
```
